```python
import os as _os
_os.environ.setdefault('JAX_PLATFORMS', 'cpu')
import jax
import jax.numpy as jnp

def _softmax(x, axis=-1):
    return jax.nn.softmax(x, axis=axis)

def _gelu(x):
    return jax.nn.gelu(x, approximate=True)

def _silu(x):
    return jax.nn.silu(x)

def _sigmoid(x):
    return jax.nn.sigmoid(x)

def _layernorm(x, axis=-1, eps=1e-05):
    m = jnp.mean(x, axis=axis, keepdims=True)
    v = jnp.var(x, axis=axis, keepdims=True)
    return (x - m) / jnp.sqrt(v + eps)

def _scatter_add(tgt, idx, src, axis=0):
    return tgt.at[idx].add(src)

def _segment_sum(src, seg, n):
    return jax.ops.segment_sum(src, seg, n)

class _Rng:

    def __init__(self, key):
        self._k = key

    def _next(self):
        self._k, sub = jax.random.split(self._k)
        return sub

    def normal(self, shape):
        return jax.random.normal(self._next(), shape, dtype=jnp.bfloat16)

    def randint(self, lo, hi, shape):
        return jax.random.randint(self._next(), shape, lo, hi, dtype=jnp.int32)

    def uniform(self, shape, lo=0.0, hi=1.0):
        return jax.random.uniform(self._next(), shape, jnp.bfloat16, lo, hi)

    def permutation(self, n):
        return jax.random.permutation(self._next(), n)
kernel_name = 'gated_mix__ssm_conv_h3__memory_aug_recurrent_mem_tr__prompt'

def setup_inputs():
    _rng = _Rng(jax.random.key(int.from_bytes(__import__("os").urandom(4), "little")))
    _w = lambda a: (lambda t: t.astype(jnp.bfloat16) if jnp.issubdtype(t.dtype, jnp.floating) else t)(jnp.asarray(a))

    def _A_setup():
        B, S, D = (1, 2048, 1024)
        ks = 4
        return {'q': _w((lambda *s: _rng.normal(s) * 0.05)(B, S, D)), 'k': _w((lambda *s: _rng.normal(s) * 0.4)(B, S, D)), 'v': _w((lambda *s: _rng.normal(s) * 0.4)(B, S, D)), 'shift_k': _w((lambda *s: _rng.normal(s) * 0.4)(D, ks) * 0.5), 'ssm_k': _w((lambda *s: _rng.normal(s) * 0.4)(D, S) * (1.0 / S ** 0.5)), 'ssm_D': _w((lambda *s: _rng.normal(s) * 0.4)(D))}
    _A_in = _A_setup()

    def _B_setup():
        B, S, Dm = (1, 2048, 1024)
        H, Dh = (32, 128)
        M, seg = (8, 32)
        seg = min(seg, S)
        S = S // seg * seg
        return {'x': _w((lambda *s: _rng.normal(s) * 0.05)(B, S, Dm)), 'mem0': _w((lambda *s: _rng.normal(s) * 0.4)(B, M, Dm)), 'Wq': _w((lambda *s: _rng.normal(s) * 3.2)(Dm, H, Dh) * Dm ** (-0.5)), 'Wk': _w((lambda *s: _rng.normal(s) * 3.2)(Dm, H, Dh) * Dm ** (-0.5)), 'Wv': _w((lambda *s: _rng.normal(s) * 0.4)(Dm, H, Dh) * Dm ** (-0.5)), 'Wo': _w((lambda *s: _rng.normal(s) * 0.4)(H, Dh, Dm) * (H * Dh) ** (-0.5)), 'seg_len': seg}
    _B_in = _B_setup()
    return {'A_q': _A_in['q'], 'A_k': _A_in['k'], 'A_v': _A_in['v'], 'A_shift_k': _A_in['shift_k'], 'A_ssm_k': _A_in['ssm_k'], 'A_ssm_D': _A_in['ssm_D'], 'B_x': _B_in['x'], 'B_mem0': _B_in['mem0'], 'B_Wq': _B_in['Wq'], 'B_Wk': _B_in['Wk'], 'B_Wv': _B_in['Wv'], 'B_Wo': _B_in['Wo'], 'B_seg_len': _B_in['seg_len'], 'gate_w': _w((lambda *s: _rng.normal(s) * 0.05)(1024) * 16.0)}

def reference(A_q, A_k, A_v, A_shift_k, A_ssm_k, A_ssm_D, B_x, B_mem0, B_Wq, B_Wk, B_Wv, B_Wo, B_seg_len, gate_w):

    def _A_ref(q, k, v, shift_k, ssm_k, ssm_D):
        B, S, D = q.shape
        ks = shift_k.shape[-1]
        k_pad = jnp.pad(k, ((0, 0), (ks - 1, 0), (0, 0)))
        k_shift = jnp.zeros_like(k)
        for t in range(ks):
            k_shift = k_shift + k_pad[:, t:t + S, :] * shift_k[:, ks - 1 - t][None, None, :]
        kv = k_shift * v
        L = 2 * S
        kv_pad = jnp.pad(kv, ((0, 0), (0, S), (0, 0)))
        kf_pad = jnp.pad(ssm_k, ((0, 0), (0, S)))
        kv_f = (lambda x, axes=(-2, -1): jnp.fft.rfft2(x.astype(jnp.float32), axes=axes))(kv_pad[:, None, :, :], axes=(1, 2))
        kf_f = (lambda x, axes=(-2, -1): jnp.fft.rfft2(x.astype(jnp.float32), axes=axes))(kf_pad[:, None, :], axes=(1, 2))
        kf_f = (lambda x, *d: x.transpose(*d))(kf_f, 1, 2, 0)
        y_f = kv_f * kf_f[None, :, :, :]
        y = (lambda x, s, axes=(-2, -1): jnp.fft.irfft2(x, s=s, axes=axes).astype(jnp.bfloat16))(y_f, (1, L), axes=(1, 2))[:, 0, :S, :]
        y = y + kv * ssm_D[None, None, :]
        return q * y

    def _B_ref(x, mem0, Wq, Wk, Wv, Wo, seg_len):
        B, S, Dm = x.shape
        H, Dh = (Wq.shape[1], Wq.shape[2])
        M = mem0.shape[1]
        scale = Dh ** (-0.5)
        n_seg = S // seg_len
        L = M + seg_len
        idx = jnp.arange(L)
        mask = (idx[:, None] < M) | (idx[:, None] >= idx[None, :])
        mem = mem0
        outs = []
        for s in range(n_seg):
            xs = x[:, s * seg_len:(s + 1) * seg_len, :].copy()
            h = jnp.concatenate([mem, xs], axis=1)
            q = jnp.einsum('btd,dhe->bhte', h, Wq)
            k = jnp.einsum('btd,dhe->bhte', h, Wk)
            v = jnp.einsum('btd,dhe->bhte', h, Wv)
            scores = jnp.einsum('bhqe,bhke->bhqk', q, k) * scale
            scores = jnp.where(mask[None, None], scores, -1000000000.0)
            p = _softmax(scores, axis=-1)
            o = jnp.einsum('bhqk,bhke->bhqe', p, v)
            o = jnp.einsum('bhte,hed->btd', o, Wo)
            mem = o[:, :M, :].copy()
            outs.append(o[:, M:, :])
        return jnp.concatenate(outs, axis=1)
    x = A_q
    g = _sigmoid((x * gate_w).sum(-1, keepdims=True))
    a = _A_ref(x, A_k, A_v, A_shift_k, A_ssm_k, A_ssm_D)
    b = _B_ref(x, B_mem0, B_Wq, B_Wk, B_Wv, B_Wo, B_seg_len)
    return g * a + (1 - g) * b
```

```python
import functools
import os

import numpy as np
import jax
import jax.numpy as jnp
from jax import lax
import jax.experimental.pallas as pl
import jax.experimental.pallas.tpu as pltpu

F32 = jnp.float32
BF16 = jnp.bfloat16

LANES = 128
CH = 128
NEG = -1000000000.0
KPAD = 16

LAG1 = int(os.environ.get("LAG1", "1"))
LAG2 = int(os.environ.get("LAG2", "4"))
KS_H = int(os.environ.get("KSH", "24"))
NPAIR_RUN = int(os.environ.get("NPAIR_RUN", "-1"))
SKIP_A = int(os.environ.get("SKIP_A", "0"))
MC = int(os.environ.get("MC", "128"))
EPI_SEGS = int(os.environ.get("EPI_SEGS", "8"))
PRO_KSPLIT = int(os.environ.get("PRO_KSPLIT", "2"))
EPI_RUN = int(os.environ.get("EPI_RUN", "-1"))
PRO_RUN = int(os.environ.get("PRO_RUN", "-1"))
NO_A_DMA = int(os.environ.get("NO_A_DMA", "0"))
PACED = int(os.environ.get("PACED", "0"))
EARLY_W = int(os.environ.get("EARLY_W", "1"))
U32 = int(os.environ.get("U32", "1"))
ANCHOR = int(os.environ.get("ANCHOR", "1"))
FWD_SLOTS = tuple(int(v) for v in os.environ.get("FWD_SLOTS", "8,22").split(","))
NO_FWD = int(os.environ.get("NO_FWD", "0"))
NO_MAC = int(os.environ.get("NO_MAC", "0"))
FWD_AT = os.environ.get("FWD_AT", "spread")


def _dft_mats():
    f = np.concatenate([np.arange(0, CH, 2), np.arange(1, CH, 2)])
    t = np.arange(CH)
    ang = np.pi * np.outer(2 * f + 1, t) / (2 * CH)
    fwd = np.concatenate([np.cos(ang), -np.sin(ang)], axis=0)
    inv = np.concatenate([np.cos(ang).T, -np.sin(ang).T], axis=1) / CH
    return fwd.astype(np.float32), inv.astype(np.float32)


def _dot(a, b):
    return jnp.dot(a, b, preferred_element_type=F32)


def _dot_nt(a, b):
    return lax.dot_general(a, b, (((1,), (1,)), ((), ())), preferred_element_type=F32)


def _make_kernel(S, D, H, E, M, SEG, KS):
    assert E == LANES and M == 8 and SEG == 32 and D % LANES == 0 and S % (2 * SEG) == 0
    NB = D // LANES
    NC = S // CH
    NSEG = S // SEG
    NPAIR = NSEG // 2
    R = NSEG * M
    HG = 8
    NG = H // HG
    NGT = 3 * NG
    scale = float(E) ** -0.5
    HALF = CH // 2
    N_EPI = NSEG // EPI_SEGS
    PPB = NPAIR // NB
    CPI = NC // PPB
    PR = 16
    SPI = (CH // PR) // PPB
    assert NPAIR % NB == 0 and NC % PPB == 0 and (CH // PR) % PPB == 0

    def kernel(x_hbm, k_hbm, v_hbm, sk_hbm, wq_hbm, wk_hbm, wv_hbm, wo_hbm,
               shift_ref, dvec_ref, gw_ref, mem0_ref, fwd_ref, inv_ref,
               out_hbm,
               x_v, k_v, v_v, sk_v, wst, wqkv, wo_s, xp, pz, odef, outb, gm,
               u_s, kk_s, kraw, zsep, sems):
        w_hbm = (wq_hbm, wk_hbm, wv_hbm)
        ZOFF = 3 * H * R if ANCHOR else 0
        zbuf = pz if ANCHOR else zsep

        def wq_load(n, lo, hi):
            if U32:
                return pltpu.bitcast(wqkv[n, lo // 2:hi // 2, :], BF16)
            return wqkv[n, lo:hi, :]

        def wo_load(j, lo, hi):
            if U32:
                return pltpu.bitcast(wo_s[j, lo // 2:hi // 2, :], BF16)
            return wo_s[j, lo:hi, :]
        wo_dst = wo_s.bitcast(BF16) if U32 else wo_s

        def cp_k(c):
            return pltpu.make_async_copy(k_hbm.at[:, pl.ds(c * LANES, LANES)],
                                         k_v.at[c, pl.ds(KPAD, S), :], sems.at[c])

        def cp_v(c):
            return pltpu.make_async_copy(v_hbm.at[:, pl.ds(c * LANES, LANES)], v_v.at[c], sems.at[NB + c])

        def cp_sk(c):
            return pltpu.make_async_copy(sk_hbm.at[pl.ds(c * LANES, LANES), :], sk_v.at[c], sems.at[2 * NB + c])

        SX = 3 * NB
        cp_x = pltpu.make_async_copy(x_hbm, x_v, sems.at[SX])
        SXP = SX + 1

        def cp_xp(s):
            return pltpu.make_async_copy(x_hbm.at[pl.ds(s * SEG, M), :], xp.at[pl.ds(s * M, M), :], sems.at[SXP])
        SW = SXP + 1

        def cp_w(m, g):
            return pltpu.make_async_copy(w_hbm[m].at[:, pl.ds(g * HG, HG), :], wst.at[m * NG + g],
                                         sems.at[SW + m * NG + g])

        def wait_w(gi):
            pltpu.make_async_copy(wst.at[gi], wst.at[gi], sems.at[SW + gi]).wait()
        SO = SW + NGT

        def cp_wo(j):
            return pltpu.make_async_copy(wo_hbm.at[:, pl.ds(j * LANES, LANES)], wo_dst.at[j], sems.at[SO + j])
        SOUT = SO + NB

        def cp_out(q):
            rows = EPI_SEGS * SEG
            r0 = pl.multiple_of(q * rows, rows)
            return pltpu.make_async_copy(outb.at[pl.ds(r0, rows), :], out_hbm.at[pl.ds(r0, rows), :],
                                         sems.at[SOUT + q])

        cp_k(0).start(); cp_v(0).start(); cp_sk(0).start()
        for s in range(NSEG):
            cp_xp(s).start()
        def late_starts():
            for gi in range(EARLY_W, NGT):
                cp_w(gi // NG, gi % NG).start()
            cp_x.start()
            for j in range(NB):
                cp_wo(j).start()
            for c in range(1, NB):
                if not NO_A_DMA:
                    cp_k(c).start(); cp_v(c).start(); cp_sk(c).start()
        for gi in range(EARLY_W):
            cp_w(gi // NG, gi % NG).start()
        if not PACED:
            late_starts()

        for c in range(NB):
            k_v[c, 0:KPAD, :] = jnp.zeros((KPAD, LANES), BF16)

        def fwd_unit(c, j, slot):
            r0 = pl.multiple_of(j * CH, CH)
            sh = shift_ref[c].astype(F32)
            kw = k_v[c, pl.ds(r0, CH + KPAD), :].astype(F32)
            ks = kw[KPAD:] * sh[0:1, :]
            for t in range(1, KS):
                ks = ks + kw[KPAD - t:KPAD - t + CH] * sh[t:t + 1, :]
            kv = (ks * v_v[c, pl.ds(r0, CH), :].astype(F32)).astype(BF16)
            skc = sk_v[c, :, pl.ds(r0, CH)]
            ub = pl.multiple_of((slot * NC + j) * 2 * CH, 2 * CH)
            u_s[pl.ds(ub, CH), :] = _dot(fwd_ref[0:CH, :], kv)
            u_s[pl.ds(ub + CH, CH), :] = _dot(fwd_ref[CH:, :], kv)
            kr = _dot_nt(fwd_ref[0:CH, :], skc)
            ki = _dot_nt(fwd_ref[CH:, :], skc)
            first = j == 0
            dv = jnp.where(first, dvec_ref[c].astype(F32), 0.0)
            pr = kraw[0:CH, :]
            pi = kraw[CH:, :]
            kk_s[slot, j, 0:HALF, :] = kr[0:HALF] - pi[0:HALF] + dv
            kk_s[slot, j, HALF:CH, :] = kr[HALF:] + pi[HALF:] + dv
            kk_s[slot, j, CH:CH + HALF, :] = ki[0:HALF] + pr[0:HALF]
            kk_s[slot, j, CH + HALF:, :] = ki[HALF:] - pr[HALF:]
            last = j == NC - 1
            kraw[0:CH, :] = jnp.where(last, 0.0, kr)
            kraw[CH:, :] = jnp.where(last, 0.0, ki)

        def make_mac(c, sl, slot, nslots):
            r0 = pl.multiple_of(sl * PR, PR)
            units = [(i, j) for i in range(NC) for j in range(i + 1)]
            st = {}

            def run(lo, hi):
                for (i, j) in units[lo:hi]:
                    ub = pl.multiple_of((slot * NC + j) * 2 * CH + r0, PR)
                    ur = u_s[pl.ds(ub, PR), :]
                    ui = u_s[pl.ds(ub + CH, PR), :]
                    kr = kk_s[slot, i - j, pl.ds(r0, PR), :]
                    ki = kk_s[slot, i - j, pl.ds(CH + r0, PR), :]
                    tr = ur * kr - ui * ki
                    ti = ur * ki + ui * kr
                    if j == 0:
                        st["r"], st["i"] = tr, ti
                    else:
                        st["r"], st["i"] = st["r"] + tr, st["i"] + ti
                    if j == i:
                        zr0 = pl.multiple_of(ZOFF + (c * NC + i) * 2 * CH + r0, PR)
                        zbuf[pl.ds(zr0, PR), :] = st["r"].astype(BF16)
                        zbuf[pl.ds(zr0 + CH, PR), :] = st["i"].astype(BF16)
            n = len(units)
            return [functools.partial(run, (n * t) // nslots, (n * (t + 1)) // nslots) for t in range(nslots)]

        kraw[...] = jnp.zeros(kraw.shape, F32)
        cp_k(0).wait(); cp_v(0).wait(); cp_sk(0).wait()

        def fwd0_body(j, c):
            fwd_unit(0, j, 0)
            return c
        lax.fori_loop(0, NC, fwd0_body, 0, unroll=2)

        def repack_piece(gi, d0, nd):
            n0 = pl.multiple_of(gi * HG, HG)
            for i in range(nd // 16):
                blk = wst[gi, d0 + i * 16:d0 + (i + 1) * 16]
                sw = jnp.swapaxes(blk, 0, 1)
                if U32:
                    wqkv[pl.ds(n0, HG), (d0 + i * 16) // 2:(d0 + (i + 1) * 16) // 2, :] = pltpu.bitcast(sw, jnp.uint32)
                else:
                    wqkv[pl.ds(n0, HG), d0 + i * 16:d0 + (i + 1) * 16, :] = sw

        for s in range(NSEG):
            cp_xp(s).wait()
        cp_w(0, 0).wait()
        if PACED:
            late_starts()

        def rp0_body(i, c):
            d0 = pl.multiple_of(i * 16, 16)
            sw = jnp.swapaxes(wst[0, pl.ds(d0, 16)], 0, 1)
            if U32:
                wqkv[0:HG, pl.ds(pl.multiple_of(i * 8, 8), 8), :] = pltpu.bitcast(sw, jnp.uint32)
            else:
                wqkv[0:HG, pl.ds(d0, 16), :] = sw
            return c
        lax.fori_loop(0, D // 16, rp0_body, 0, unroll=4)

        def pro_body(it, c):
            nxt = jnp.minimum(it + 1, NGT - 1)

            @pl.when(it + 1 < NGT)
            def _():
                wait_w(it + 1)
            nr = R // MC
            nk = PRO_KSPLIT
            kw = D // nk
            pd = D // (HG * nr * nk)
            for hh in range(HG):
                n = it * HG + hh
                for r in range(nr):
                    acc = None
                    for kk in range(nk):
                        t = _dot(xp[r * MC:(r + 1) * MC, kk * kw:(kk + 1) * kw], wq_load(n, kk * kw, (kk + 1) * kw))
                        acc = t if acc is None else t + acc
                        repack_piece(nxt, ((hh * nr + r) * nk + kk) * pd, pd)
                    pz[pl.ds(pl.multiple_of(n * R + r * MC, MC), MC), :] = acc.astype(BF16)
            return c
        npro = NGT if PRO_RUN < 0 else PRO_RUN
        lax.fori_loop(0, npro, pro_body, 0)
        for gi in range(min(npro + 1, NGT), NGT):
            wait_w(gi)

        cp_x.wait()
        for j in range(NB):
            cp_wo(j).wait()

        L = SEG + 2 * M
        ri = lax.broadcasted_iota(jnp.int32, (L, L), 0)
        ci = lax.broadcasted_iota(jnp.int32, (L, L), 1)

        def masks(par):
            off = SEG + M * par

            def pos(i):
                return jnp.where(i < M, i, jnp.where(i < SEG, i + M, i - off + M))

            def valid(i):
                return (i < SEG) | ((i >= off) & (i < off + M))
            allowed = valid(ci) & ((ri < M) | (pos(ri) >= pos(ci)) | jnp.logical_not(valid(ri)))
            fill = jnp.where(valid(ci), NEG, -jnp.inf).astype(F32)
            return allowed, fill

        def pair_body(p, mem):
            cb = p // PPB
            ph = p % PPB
            cn = jnp.minimum(cb + 1, NB - 1)
            if not SKIP_A:
                @pl.when((ph == 0) & (cb + 1 < NB))
                def _():
                    cp_k(cb + 1).wait(); cp_v(cb + 1).wait(); cp_sk(cb + 1).wait()
            slot = cb % 2
            a_work = []
            if not SKIP_A and not NO_FWD:
                for t in range(CPI):
                    a_work.append(functools.partial(fwd_unit, cn, ph * CPI + t, 1 - slot))
            m_work = []
            if not SKIP_A and not NO_MAC:
                for t in range(SPI):
                    m_work.append(make_mac(cb, ph * SPI + t, slot, H))

            prow = pl.multiple_of(p * 2 * M, 2 * M)
            gw = gw_ref[...].astype(F32)
            defs = []
            for par in range(2):
                allowed, fill = masks(par)
                r0 = pl.multiple_of(p * 2 * SEG + par * SEG, SEG)
                xin = x_v[pl.ds(r0, SEG), :].astype(F32)
                lhs = jnp.concatenate([mem, xin[M:]], axis=0).astype(BF16)
                z = jnp.sum(xin * gw, axis=1, keepdims=True)
                g = jnp.broadcast_to(1.0 / (1.0 + jnp.exp(-z)), (SEG, LANES))
                gm[pl.ds(r0, SEG), :] = g
                o_in = [None] * H
                o_df = [None] * H
                QKV = {}
                EL = {}

                def do_qkv(h):
                    qkv = []
                    for m in range(3):
                        t = _dot(lhs, wq_load(m * H + h, 0, D))
                        pt = pz[pl.ds(pl.multiple_of((m * H + h) * R + prow, 2 * M), 2 * M), :]
                        qkv.append(jnp.concatenate([t, pt.astype(F32)], axis=0).astype(BF16))
                    QKV[h] = qkv

                def do_scores(h):
                    q, k, _ = QKV[h]
                    s = _dot_nt(q, k) * scale
                    s = jnp.where(allowed, s, fill)
                    mx = jnp.max(s, axis=1, keepdims=True)
                    e = jnp.exp(s - mx)
                    l = jnp.sum(e, axis=1, keepdims=True)
                    EL[h] = (e.astype(BF16), l)

                def do_pv(h):
                    e, l = EL[h]
                    o = _dot(e, QKV[h][2]) * pl.reciprocal(l, approx=True)
                    o_in[h] = o[0:SEG].astype(BF16)
                    ob = 2 * NC * 2 * CH + (h * 2 + par) * M
                    u_s[ob:ob + M, :] = o[SEG + M * par:SEG + M * par + M]

                def wo_part(j, h0, h1, acc):
                    for h in range(h0, h1):
                        t = _dot(o_in[h], wo_load(j, h * E, (h + 1) * E))
                        acc = t if acc is None else t + acc
                    return acc

                mine_a = a_work[par * len(a_work) // 2:(par + 1) * len(a_work) // 2]
                mine_m = m_work[par * len(m_work) // 2:(par + 1) * len(m_work) // 2]
                res1 = [None] * NB
                oc1 = None
                for t in range(H + LAG2):
                    if t < H:
                        do_qkv(t)
                    else:
                        res1[t - H] = wo_part(t - H, 0, KS_H, None)
                    if 0 <= t - LAG1 < H:
                        do_scores(t - LAG1)
                    if 0 <= t - LAG2 < H:
                        do_pv(t - LAG2)
                    if 0 <= t - LAG2 < H:
                        for pieces in mine_m:
                            pieces[t - LAG2]()
                    if FWD_AT == "spread" and t in FWD_SLOTS and mine_a:
                        mine_a[FWD_SLOTS.index(t)]()
                for j in range(LAG2, NB):
                    res1[j] = wo_part(j, 0, KS_H, None)
                defs.append(o_df)
                res = [wo_part(j, KS_H, H, res1[j]) for j in range(NB)]
                if FWD_AT == "end":
                    for w in mine_a:
                        w()
                res = jnp.concatenate(res, axis=1)
                mem = res[0:M].astype(BF16).astype(F32)
                g1 = jnp.concatenate([1.0 - g] * NB, axis=1)
                outb[pl.ds(r0 + M, SEG - M), :] = (g1 * res)[M:].astype(BF16)
            for h in range(H):
                ob = 2 * NC * 2 * CH + h * 2 * M
                odef[pl.ds(prow, 2 * M), h * E:(h + 1) * E] = u_s[ob:ob + 2 * M, :].astype(BF16)
            return mem

        lax.fori_loop(0, NPAIR if NPAIR_RUN < 0 else NPAIR_RUN, pair_body, mem0_ref[...].astype(F32))
        if NPAIR_RUN >= 0 or SKIP_A:
            done = 0 if SKIP_A else max(0, (min(NPAIR_RUN, NPAIR) + PPB - 1) // PPB) if NPAIR_RUN >= 0 else NB - 1
            for c in range(1 + min(done, NB - 1), NB):
                if not NO_A_DMA:
                    cp_k(c).wait(); cp_v(c).wait(); cp_sk(c).wait()

        ER = EPI_SEGS * M
        ROWS = EPI_SEGS * SEG

        def epi_body(q, c):
            e0 = pl.multiple_of(q * ER, ER)
            r0 = pl.multiple_of(q * ROWS, ROWS)
            od = odef[pl.ds(e0, ER), :]
            iv = inv_ref[...]
            g = gm[pl.ds(r0, ROWS), :]
            for j in range(NB):
                lo, hi = j * LANES, (j + 1) * LANES
                res = _dot(od, wo_load(j, 0, H * E))
                ys = [_dot(iv, zbuf[pl.ds(pl.multiple_of(ZOFF + (j * NC + q * (ROWS // CH) + i) * 2 * CH, 2 * CH), 2 * CH), :]) for i in range(ROWS // CH)]
                y = jnp.concatenate(ys, axis=0)
                a = g * (x_v[pl.ds(r0, ROWS), lo:hi].astype(F32) * y)
                bb = outb[pl.ds(r0, ROWS), lo:hi].astype(F32)
                parts = []
                for sgm in range(EPI_SEGS):
                    s0 = sgm * SEG
                    parts.append((1.0 - g[s0:s0 + M]) * res[sgm * M:(sgm + 1) * M])
                    parts.append(bb[s0 + M:s0 + SEG])
                bfull = jnp.concatenate(parts, axis=0)
                outb[pl.ds(r0, ROWS), lo:hi] = (a + bfull).astype(BF16)
            cp_out(q).start()
            return c
        ne = N_EPI if EPI_RUN < 0 else EPI_RUN
        lax.fori_loop(0, ne, epi_body, 0)
        for q in range(ne):
            cp_out(q).wait()

    n_sems = 3 * NB + 2 + NGT + NB + N_EPI
    scratch = [
        pltpu.VMEM((S, D), BF16),
        pltpu.VMEM((NB, S + KPAD, LANES), BF16),
        pltpu.VMEM((NB, S, LANES), BF16),
        pltpu.VMEM((NB, LANES, S), BF16),
        pltpu.VMEM((NGT, D, HG, E), BF16),
        pltpu.VMEM((3 * H, D // 2, E), jnp.uint32) if U32 else pltpu.VMEM((3 * H, D, E), BF16),
        pltpu.VMEM((NB, H * E // 2, LANES), jnp.uint32) if U32 else pltpu.VMEM((NB, H * E, LANES), BF16),
        pltpu.VMEM((R, D), BF16),
        pltpu.VMEM((3 * H * R + (NB * NC * 2 * CH if ANCHOR else 0), E), BF16),
        pltpu.VMEM((R, H * E), BF16),
        pltpu.VMEM((S, D), BF16),
        pltpu.VMEM((S, LANES), F32),
        pltpu.VMEM((2 * NC * 2 * CH + 2 * H * M, LANES), F32),
        pltpu.VMEM((2, NC, 2 * CH, LANES), F32),
        pltpu.VMEM((2 * CH, LANES), F32),
        pltpu.VMEM((16 if ANCHOR else NB * NC * 2 * CH, LANES), BF16),
        pltpu.SemaphoreType.DMA((n_sems,)),
    ]
    return kernel, scratch


@functools.partial(jax.jit, static_argnames=("B_seg_len",))
def pallas_gated_mix__ssm_conv_h3__memory_aug_recurrent_mem_tr__prompt_kernel(
    A_q, A_k, A_v, A_shift_k, A_ssm_k, A_ssm_D, B_x, B_mem0, B_Wq, B_Wk, B_Wv, B_Wo, B_seg_len, gate_w,
):
    B, S, D = A_q.shape
    assert B == 1
    H, E = B_Wq.shape[1], B_Wq.shape[2]
    M = B_mem0.shape[1]
    KS = A_shift_k.shape[1]
    NB = D // LANES
    kernel, scratch = _make_kernel(S, D, H, E, M, int(B_seg_len), KS)
    fwd, inv = _dft_mats()

    any_spec = pl.BlockSpec(memory_space=pl.ANY)
    vmem_spec = pl.BlockSpec(memory_space=pltpu.VMEM)
    out = pl.pallas_call(
        kernel,
        out_shape=jax.ShapeDtypeStruct((S, D), A_q.dtype),
        in_specs=[any_spec] * 8 + [vmem_spec] * 6,
        out_specs=any_spec,
        scratch_shapes=scratch,
        compiler_params=pltpu.CompilerParams(vmem_limit_bytes=124 * 1024 * 1024),
    )(
        A_q.reshape(S, D), A_k.reshape(S, D), A_v.reshape(S, D), A_ssm_k,
        B_Wq, B_Wk, B_Wv, B_Wo.reshape(H * E, D),
        A_shift_k.reshape(NB, LANES, KS).transpose(0, 2, 1), A_ssm_D.reshape(NB, 1, LANES),
        gate_w.reshape(1, D), B_mem0.reshape(M, D),
        jnp.asarray(fwd, dtype=BF16), jnp.asarray(inv, dtype=BF16),
    )
    return out.reshape(1, S, D)
```

```python
import functools

import numpy as np
import jax
import jax.numpy as jnp
from jax import lax
import jax.experimental.pallas as pl
import jax.experimental.pallas.tpu as pltpu

F32 = jnp.float32
BF16 = jnp.bfloat16
U32 = jnp.uint32

LANES = 128
CH = 128
PR = 16
MB = 2
NEG = -1000000000.0
KPAD = 16
KOFS = 64
HG = 8
MC = 128
HP = 2
LAG1 = 1
LAG2 = 2
KS_H = 24
KSPL = 2
EPI_SEGS = 8
NP1 = 2


def _dft_mats():
    f = np.concatenate([np.arange(0, CH, 2), np.arange(1, CH, 2)])
    t = np.arange(CH)
    ang = np.pi * np.outer(2 * f + 1, t) / (2 * CH)
    fwd = np.concatenate([np.cos(ang), -np.sin(ang)], axis=0)
    inv = np.concatenate([np.cos(ang).T, -np.sin(ang).T], axis=1) / CH
    return fwd.astype(np.float32), inv.astype(np.float32)


def _dot(a, b):
    return jnp.dot(a, b, preferred_element_type=F32)


def _dot_nt(a, b):
    return lax.dot_general(a, b, (((1,), (1,)), ((), ())), preferred_element_type=F32)


def _split(n, parts):
    return [((n * t) // parts, (n * (t + 1)) // parts) for t in range(parts)]


def _make_kernel(S, D, H, E, M, SEG, KS):
    assert E == LANES and M == 8 and SEG == 32 and D % LANES == 0 and S % (4 * SEG) == 0
    assert KS - 1 <= KPAD and H % HG == 0 and H % HP == 0
    NB = D // LANES
    NC = S // CH
    NSEG = S // SEG
    NPAIR = NSEG // 2
    R = NSEG * M
    NG = H // HG
    NGT = 3 * NG
    scale = float(E) ** -0.5
    HALF = CH // 2
    N_EPI = NSEG // EPI_SEGS
    SPB = CH // PR
    assert NB * SPB == NSEG
    UPI = -(-NB * NC // (NGT - NP1))
    assert UPI <= NC
    WROWS = D // 2
    UOFF = 3 * H * (R // 2)
    KOFF = UOFF + NB * NC * 2 * CH
    OOFF = KOFF + NB * NC * 2 * CH
    AROWS = OOFF + 2 * H * M
    NR = R // MC
    NSLOT = HG * NR * 2

    SA = 0
    SW = SA + NB
    SS = SW + NGT
    SX = SS + 1
    SOUT = SX + 1
    n_sems = SOUT + 1

    def kernel(x_hbm, k_hbm, v_hbm, sk_hbm, wq_hbm, wk_hbm, wv_hbm, wo_hbm,
               shift_hbm, dvec_hbm, gw_hbm, mem0_hbm, fwd_hbm, inv_hbm,
               out_hbm,
               x_v, wqkv, wo_s, ar, gm, shift_ref, dvec_ref, gw_ref, mem0_ref, fwd_ref, inv_ref, sems):
        w_hbm = (wq_hbm, wk_hbm, wv_hbm)

        def wq_load(n, lo, hi):
            return pltpu.bitcast(wqkv[n, lo // 2:hi // 2, :], BF16)

        def wo_load(j, lo, hi):
            return wo_s[j, lo:hi, :]

        def rows(row, n, align):
            return pl.ds(row if isinstance(row, int) else pl.multiple_of(row, align), n)

        def ld_f32(row, n, align):
            return lax.bitcast_convert_type(ar[rows(row, n, align), :], F32)

        def st_f32(row, val, align):
            ar[rows(row, val.shape[0], align), :] = lax.bitcast_convert_type(val, U32)

        def ld_bf(row, n, align):
            return pltpu.bitcast(ar[rows(row, n, align), :], BF16)

        def st_bf(row, val, align):
            ar[rows(row, val.shape[0] // 2, align), :] = pltpu.bitcast(val, U32)

        cp_x = pltpu.make_async_copy(x_hbm, x_v, sems.at[SX])

        def cp_wo(j):
            return pltpu.make_async_copy(wo_hbm.at[:, pl.ds(j * LANES, LANES)], wo_s.at[j], sems.at[SX])

        def prologue(k_v, v_v, sk_v, wst, xp, xpu, dv_s):
            def cp_a(c):
                return [
                    pltpu.make_async_copy(k_hbm.at[:, pl.ds(c * LANES, LANES)], k_v.at[c, pl.ds(KOFS, S), :],
                                          sems.at[SA + c]),
                    pltpu.make_async_copy(v_hbm.at[:, pl.ds(c * LANES, LANES)], v_v.at[c], sems.at[SA + c]),
                    pltpu.make_async_copy(sk_hbm.at[pl.ds(c * LANES, LANES), :], sk_v.at[c], sems.at[SA + c]),
                ]

            def cp_w(gi):
                return pltpu.make_async_copy(w_hbm[gi // NG].at[:, pl.ds((gi % NG) * HG, HG), :], wst.at[gi],
                                             sems.at[SW + gi])

            def wait_w(gi):
                pltpu.make_async_copy(wst.at[gi], wst.at[gi], sems.at[SW + gi]).wait()

            small = [pltpu.make_async_copy(x_hbm.at[pl.ds(s * SEG, M), :], xp.at[pl.ds(s * M, M), :], sems.at[SS])
                     for s in range(NSEG)]
            small += [pltpu.make_async_copy(src, dst, sems.at[SS]) for src, dst in (
                (shift_hbm, shift_ref), (dvec_hbm, dvec_ref), (gw_hbm, gw_ref), (mem0_hbm, mem0_ref),
                (fwd_hbm, fwd_ref), (inv_hbm, inv_ref))]

            def bmax(it):
                return (UPI * (it - NP1 + 1) - 1) // NC

            late = []
            nxt_a = 0
            for gi in range(1, NGT):
                late.append(cp_w(gi))
                while nxt_a < NB and gi - 1 >= NP1 and nxt_a <= bmax(gi - 1):
                    late += cp_a(nxt_a)
                    nxt_a += 1
            assert nxt_a == NB
            late.append(cp_x)
            late += [cp_wo(j) for j in range(NB)]

            cp_w(0).start()
            for cp in small + late[:2]:
                cp.start()

            for c in range(NB):
                k_v[c, KOFS - KPAD:KOFS, :] = jnp.zeros((KPAD, LANES), BF16)

            def dft_unit(u):
                c = u // NC
                j = u % NC
                r0 = pl.multiple_of(j * CH, CH)
                sh = shift_ref[c].astype(F32)
                kw = k_v[c, pl.ds(r0 + (KOFS - KPAD), CH + KPAD), :].astype(F32)
                ks = kw[KPAD:] * sh[0:1, :]
                for t in range(1, KS):
                    ks = ks + kw[KPAD - t:KPAD - t + CH] * sh[t:t + 1, :]
                kv = (ks * v_v[c, pl.ds(r0, CH), :].astype(F32)).astype(BF16)
                skc = sk_v[c, :, pl.ds(r0, CH)]
                off = u * 2 * CH
                st_f32(UOFF + off, _dot(fwd_ref[0:CH, :], kv), CH)
                st_f32(UOFF + off + CH, _dot(fwd_ref[CH:, :], kv), CH)
                dv = jnp.where(j == 0, dv_s[pl.ds(c, 1), :], 0.0)
                st_f32(KOFF + off, _dot_nt(fwd_ref[0:CH, :], skc) + dv, CH)
                st_f32(KOFF + off + CH, _dot_nt(fwd_ref[CH:, :], skc), CH)

            def repack_blk(gi, i):
                blk = wst[gi, rows(i * 16, 16, 16)]
                wqkv[pl.ds(gi * HG, HG), rows(i * 8, 8, 8), :] = pltpu.bitcast(jnp.swapaxes(blk, 0, 1), U32)

            cp_w(0).wait()

            def rp0_body(i, c):
                repack_blk(0, i)
                return c
            lax.fori_loop(0, D // 16, rp0_body, 0, unroll=4)

            for cp in late[2:]:
                cp.start()
            for cp in small:
                cp.wait()
            dv_s[...] = dvec_ref[...].astype(F32)

            def xp_body(i, c):
                xr = xp[pl.ds(pl.multiple_of(i * 32, 32), 32), :]
                for kt in range(NB):
                    xpu[kt, pl.ds(pl.multiple_of(i * 16, 16), 16), :] = pltpu.bitcast(
                        xr[:, kt * LANES:(kt + 1) * LANES], U32)
                return c
            lax.fori_loop(0, R // 32, xp_body, 0)

            def pro_body(with_dft, it, c):
                nxt = jnp.minimum(it + 1, NGT - 1)
                rp0 = 0 if with_dft else NSLOT // 2
                upos = [lo for lo, _ in _split(NSLOT, UPI)] if with_dft else []
                busy = [p + d for p in upos for d in (0, 1)]
                rslots = [t for t in range(rp0, NSLOT) if t not in busy]
                rp = dict(zip(rslots, _split(D // 16, len(rslots))))
                if with_dft:
                    @pl.when((bmax(it) < NB) & ((it == NP1) | (bmax(it) != bmax(it - 1))))
                    def _():
                        for cp in cp_a(bmax(it)):
                            cp.wait()
                acc = None
                for sl in range(NSLOT):
                    hh, r, kk = sl // (2 * NR), (sl // 2) % NR, sl % 2
                    n = it * HG + hh
                    if sl == rp0:
                        @pl.when(it + 1 < NGT)
                        def _():
                            wait_w(it + 1)
                    for kt in range(kk * NB // 2, (kk + 1) * NB // 2):
                        lhs = pltpu.bitcast(xpu[kt, r * (MC // 2):(r + 1) * (MC // 2), :], BF16)
                        d = _dot(lhs, wq_load(n, kt * LANES, (kt + 1) * LANES))
                        acc = d if acc is None else d + acc
                    if kk == 1:
                        st_bf(n * (R // 2) + r * (MC // 2), acc.astype(BF16), MC // 2)
                        acc = None
                    if sl in rp:
                        for i in range(*rp[sl]):
                            repack_blk(nxt, i)
                    if sl in upos:
                        dft_unit(jnp.minimum(UPI * (it - NP1) + upos.index(sl), NB * NC - 1))
                return c
            lax.fori_loop(0, NP1, functools.partial(pro_body, False), 0)
            lax.fori_loop(NP1, NGT, functools.partial(pro_body, True), 0)

        pl.run_scoped(
            prologue,
            pltpu.VMEM((NB, S + KOFS, LANES), BF16),
            pltpu.VMEM((NB, S, LANES), BF16),
            pltpu.VMEM((NB, LANES, S), BF16),
            pltpu.VMEM((NGT, D, HG, E), BF16),
            pltpu.VMEM((R, D), BF16),
            pltpu.VMEM((NB, R // 2, LANES), U32),
            pltpu.VMEM((NB, LANES), F32),
        )

        def main(outb):
            cp_x.wait()
            for j in range(NB):
                cp_wo(j).wait()

            def cp_out(q):
                nrow = EPI_SEGS * SEG
                r0 = pl.multiple_of(q * nrow, nrow)
                return pltpu.make_async_copy(outb.at[pl.ds(r0, nrow), :], out_hbm.at[pl.ds(r0, nrow), :],
                                             sems.at[SOUT])

            mac_steps = [(i0, j) for i0 in range(NC - MB, -1, -MB) for j in range(i0 + MB)]
            cum = np.cumsum([0] + [sum(1 for i in range(i0, i0 + MB) if i >= j) for i0, j in mac_steps])

            def make_mac(p, par, nparts):
                dyn = pl.multiple_of((p // (SPB // 2)) * NC * 2 * CH + (p % (SPB // 2)) * 2 * PR, 2 * PR)
                base = par * PR
                acc = {}
                kc = {}

                def ld(off):
                    return lax.bitcast_convert_type(ar[pl.ds(dyn + off, PR), :], F32)

                def run(lo, hi):
                    for (i0, j) in mac_steps[lo:hi]:
                        if j == 0:
                            kc.clear()
                        ur = ld(UOFF + base + j * 2 * CH)
                        ui = ld(UOFF + base + j * 2 * CH + CH)
                        for i in range(max(i0, j), i0 + MB):
                            m = i - j
                            if m not in kc:
                                kc[m] = (ld(KOFF + base + m * 2 * CH), ld(KOFF + base + m * 2 * CH + CH))
                            kr, ki = kc[m]
                            tr = ur * kr - ui * ki
                            ti = ur * ki + ui * kr
                            acc[i] = (tr, ti) if j == 0 else (acc[i][0] + tr, acc[i][1] + ti)
                        if j == i0 + MB - 1:
                            for i in range(i0, i0 + MB):
                                yr, yi = acc.pop(i)
                                row = dyn + UOFF + base + i * 2 * CH
                                ar[pl.ds(row, PR), :] = lax.bitcast_convert_type(yr, U32)
                                ar[pl.ds(row + CH, PR), :] = lax.bitcast_convert_type(yi, U32)
                cuts = [int(np.searchsorted(cum, cum[-1] * t / nparts)) for t in range(nparts)] + [len(mac_steps)]
                return [functools.partial(run, cuts[t], cuts[t + 1]) for t in range(nparts)]

            def masks(par):
                nq = SEG + 2 * M * par
                nk = SEG + 2 * M + 2 * M * par
                ri = lax.broadcasted_iota(jnp.int32, (nq, nk), 0)
                ci = lax.broadcasted_iota(jnp.int32, (nq, nk), 1)
                off = SEG + M * par

                def pos(i):
                    return jnp.where(i < M, i, jnp.where(i < SEG, i + M, i - off + M))

                valid = (ci < SEG) | ((ci >= off) & (ci < off + M))
                allowed = valid & ((ri < M) | (pos(ri) >= pos(ci)))
                if par == 1:
                    other = (ri >= SEG) & (ri < SEG + M)
                    mine = jnp.logical_not(other)
                    mem_a = (ci >= SEG + 2 * M) & (ci < SEG + 3 * M)
                    xa_lo = (ci >= SEG) & (ci < SEG + M)
                    xa_hi = ci >= SEG + 3 * M
                    valid = (other & (mem_a | xa_lo | xa_hi)) | (mine & valid)
                    allowed = (other & (mem_a | (xa_lo & (ri >= ci)))) | (mine & allowed)
                fill = jnp.where(valid, NEG, -jnp.inf).astype(F32)
                return allowed, fill

            def pair_body(p, mem):
                gw = gw_ref[...].astype(F32)
                for par in range(2):
                    allowed, fill = masks(par)
                    mac = make_mac(p, par, 2 * H)
                    r0 = pl.multiple_of(p * 2 * SEG + par * SEG, SEG)
                    xin = x_v[pl.ds(r0, SEG), :].astype(F32)
                    lhs = jnp.concatenate([mem, xin[M:]], axis=0).astype(BF16)
                    zp = xin[:, 0:LANES] * gw[0:1, :]
                    for kt in range(1, NB):
                        zp = zp + xin[:, kt * LANES:(kt + 1) * LANES] * gw[kt:kt + 1, :]
                    z = jnp.sum(zp, axis=1, keepdims=True)
                    g = jnp.broadcast_to(1.0 / (1.0 + jnp.exp(-z)), (SEG, LANES))
                    gm[pl.ds(r0, SEG), :] = g
                    o_in = [None] * H
                    qkv = {}
                    prob = {}

                    first = {(h, m): _dot(lhs[:, :D // 2], wq_load(m * H + h, 0, D // 2))
                             for h in range(KSPL) for m in range(3)}

                    def do_qkv(h):
                        out = []
                        for m in range(3):
                            if (h, m) in first:
                                t = _dot(lhs[:, D // 2:], wq_load(m * H + h, D // 2, D)) + first[(h, m)]
                            else:
                                t = _dot(lhs, wq_load(m * H + h, 0, D))
                            parts = [t]
                            if m > 0 or par == 1:
                                parts.append(ld_bf((m * H + h) * (R // 2) + p * M, M, M).astype(F32))
                            if m > 0:
                                sr = OOFF + (h * 2 + m - 1) * M
                                if par == 0:
                                    st_bf(sr, t[0:2 * M].astype(BF16), M)
                                else:
                                    parts.append(ld_bf(sr, M, M).astype(F32))
                                    st_f32(sr, t[0:M], M)
                                mac[2 * h + m - 1]()
                            out.append(jnp.concatenate(parts, axis=0).astype(BF16))
                        qkv[h] = out

                    def do_scores(h):
                        q, k, _ = qkv[h]
                        s = jnp.where(allowed, _dot_nt(q, k) * scale, fill)
                        e = jnp.exp(s - jnp.max(s, axis=1, keepdims=True))
                        l = jnp.sum(e, axis=1, keepdims=True)
                        prob[h] = (e * pl.reciprocal(l, approx=True)).astype(BF16)

                    def do_pv(h):
                        o = _dot(prob[h], qkv[h][2])
                        o_in[h] = o[0:SEG].astype(BF16)
                        if par == 1:
                            st_bf(h * (R // 2) + p * M, o[SEG:].astype(BF16), M)

                    def wo_part(j, h0, h1, acc):
                        for h in range(h0, h1):
                            t = _dot(o_in[h], wo_load(j, h * E, (h + 1) * E))
                            acc = t if acc is None else t + acc
                        return acc

                    res1 = []
                    for t in range(H // HP + LAG2):
                        for u in range(HP):
                            if t < H // HP:
                                do_qkv(t * HP + u)
                            elif len(res1) < NB:
                                res1.append(wo_part(len(res1), 0, KS_H, None))
                        if 0 <= t - LAG1 < H // HP:
                            for u in range(HP):
                                do_scores((t - LAG1) * HP + u)
                        if 0 <= t - LAG2 < H // HP:
                            for u in range(HP):
                                do_pv((t - LAG2) * HP + u)
                    while len(res1) < NB:
                        res1.append(wo_part(len(res1), 0, KS_H, None))
                    res = jnp.concatenate([wo_part(j, KS_H, H, res1[j]) for j in range(NB)], axis=1)
                    mem = res[0:M].astype(BF16).astype(F32)
                    g1 = jnp.concatenate([1.0 - g] * NB, axis=1)
                    outb[pl.ds(r0 + M, SEG - M), :] = (g1 * res)[M:].astype(BF16)
                return mem

            lax.fori_loop(0, NPAIR, pair_body, mem0_ref[...].astype(F32), unroll=2)

            ER = EPI_SEGS * M
            ROWS = EPI_SEGS * SEG

            def epi_body(q, c):
                r0 = pl.multiple_of(q * ROWS, ROWS)
                od = [ld_bf(h * (R // 2) + q * (ER // 2), ER // 2, ER // 2) for h in range(H)]
                iv = inv_ref[...]
                g = gm[pl.ds(r0, ROWS), :]
                for j in range(NB):
                    lo, hi = j * LANES, (j + 1) * LANES
                    res = None
                    for h in range(H):
                        t = _dot(od[h], wo_load(j, h * E, (h + 1) * E))
                        res = t if res is None else t + res
                    i0 = q * (ROWS // CH)
                    prev = ld_f32(UOFF + (j * NC + jnp.maximum(i0 - 1, 0)) * 2 * CH, 2 * CH, CH)
                    prev = jnp.where(i0 > 0, prev, 0.0)
                    ys = []
                    for i in range(ROWS // CH):
                        cur = ld_f32(UOFF + (j * NC + i0 + i) * 2 * CH, 2 * CH, CH)
                        z = jnp.concatenate([cur[0:HALF] - prev[CH:CH + HALF],
                                             cur[HALF:CH] + prev[CH + HALF:],
                                             cur[CH:CH + HALF] + prev[0:HALF],
                                             cur[CH + HALF:] - prev[HALF:CH]], axis=0).astype(BF16)
                        ys.append(_dot(iv, z))
                        prev = cur
                    y = jnp.concatenate(ys, axis=0)
                    a = g * (x_v[pl.ds(r0, ROWS), lo:hi].astype(F32) * y)
                    parts = []
                    for sgm in range(EPI_SEGS):
                        s0 = sgm * SEG
                        parts.append((1.0 - g[s0:s0 + M]) * res[sgm * M:(sgm + 1) * M])
                        parts.append(outb[pl.ds(r0 + s0 + M, SEG - M), lo:hi].astype(F32))
                    outb[pl.ds(r0, ROWS), lo:hi] = (a + jnp.concatenate(parts, axis=0)).astype(BF16)
                cp_out(q).start()
                return c
            lax.fori_loop(0, N_EPI, epi_body, 0, unroll=2)
            for q in range(N_EPI):
                cp_out(q).wait()

        pl.run_scoped(main, pltpu.VMEM((S, D), BF16))

    scratch = [
        pltpu.VMEM((S, D), BF16),
        pltpu.VMEM((3 * H, WROWS, LANES), U32),
        pltpu.VMEM((NB, H * E, LANES), BF16),
        pltpu.VMEM((AROWS, LANES), U32),
        pltpu.VMEM((S, LANES), F32),
        pltpu.VMEM((NB, KS, LANES), BF16),
        pltpu.VMEM((NB, LANES), BF16),
        pltpu.VMEM((NB, LANES), BF16),
        pltpu.VMEM((M, D), BF16),
        pltpu.VMEM((2 * CH, CH), BF16),
        pltpu.VMEM((CH, 2 * CH), BF16),
        pltpu.SemaphoreType.DMA((n_sems,)),
    ]
    return kernel, scratch


@functools.partial(jax.jit, static_argnames=("B_seg_len",))
def pallas_gated_mix__ssm_conv_h3__memory_aug_recurrent_mem_tr__prompt_kernel(
    A_q: jax.Array,
    A_k: jax.Array,
    A_v: jax.Array,
    A_shift_k: jax.Array,
    A_ssm_k: jax.Array,
    A_ssm_D: jax.Array,
    B_x: jax.Array,
    B_mem0: jax.Array,
    B_Wq: jax.Array,
    B_Wk: jax.Array,
    B_Wv: jax.Array,
    B_Wo: jax.Array,
    B_seg_len: int,
    gate_w: jax.Array,
):
    B, S, D = A_q.shape
    assert B == 1
    H, E = B_Wq.shape[1], B_Wq.shape[2]
    M = B_mem0.shape[1]
    KS = A_shift_k.shape[1]
    NB = D // LANES
    kernel, scratch = _make_kernel(S, D, H, E, M, int(B_seg_len), KS)
    fwd, inv = _dft_mats()

    any_spec = pl.BlockSpec(memory_space=pl.ANY)
    out = pl.pallas_call(
        kernel,
        out_shape=jax.ShapeDtypeStruct((S, D), A_q.dtype),
        in_specs=[any_spec] * 14,
        out_specs=any_spec,
        scratch_shapes=scratch,
        compiler_params=pltpu.CompilerParams(vmem_limit_bytes=126 * 1024 * 1024),
    )(
        A_q.reshape(S, D), A_k.reshape(S, D), A_v.reshape(S, D), A_ssm_k,
        B_Wq, B_Wk, B_Wv, B_Wo.reshape(H * E, D),
        A_shift_k.reshape(NB, LANES, KS).transpose(0, 2, 1), A_ssm_D.reshape(NB, LANES),
        gate_w.reshape(NB, LANES), B_mem0.reshape(M, D),
        jnp.asarray(fwd, dtype=BF16), jnp.asarray(inv, dtype=BF16),
    )
    return out.reshape(1, S, D)
```

```python
import functools

import numpy as np
import jax
import jax.numpy as jnp
from jax import lax
import jax.experimental.pallas as pl
import jax.experimental.pallas.tpu as pltpu

F32 = jnp.float32
BF16 = jnp.bfloat16
U32 = jnp.uint32

LANES = 128
CH = 128
PR = 16
MB = 2
NEG = -1000000000.0
KPAD = 16
KOFS = 64
HG = 8
MC = 128
HP = 2
LAG1 = 1
LAG2 = 2
KS_H = 24
KSPL = 2
OUTJ = 2
EPI_SEGS = 8
ARING = 4
NP1 = 4


def _dft_mats():
    f = np.concatenate([np.arange(0, CH, 2), np.arange(1, CH, 2)])
    t = np.arange(CH)
    ang = np.pi * np.outer(2 * f + 1, t) / (2 * CH)
    fwd = np.concatenate([np.cos(ang), -np.sin(ang)], axis=0)
    inv = np.concatenate([np.cos(ang).T, -np.sin(ang).T], axis=1) / CH
    return fwd.astype(np.float32), inv.astype(np.float32)


def _dot(a, b):
    return jnp.dot(a, b, preferred_element_type=F32)


def _dot_nt(a, b):
    return lax.dot_general(a, b, (((1,), (1,)), ((), ())), preferred_element_type=F32)


def _split(n, parts):
    return [((n * t) // parts, (n * (t + 1)) // parts) for t in range(parts)]


def _make_kernel(S, D, H, E, M, SEG, KS):
    assert E == LANES and M == 8 and SEG == 32 and D % LANES == 0 and S % (4 * SEG) == 0
    assert KS - 1 <= KPAD and H % HG == 0 and H % HP == 0
    NB = D // LANES
    NC = S // CH
    NSEG = S // SEG
    NPAIR = NSEG // 2
    R = NSEG * M
    NG = H // HG
    NGT = 3 * NG
    scale = float(E) ** -0.5
    HALF = CH // 2
    N_EPI = NSEG // EPI_SEGS
    SPB = CH // PR
    assert NB * SPB == NSEG
    assert NGT - NP1 == NB
    WROWS = D // 2
    WPJ = H * E // D
    UOFF = 3 * H * (R // 2)
    KOFF = UOFF + NB * NC * 2 * CH
    OOFF = KOFF + NB * NC * 2 * CH
    AROWS = OOFF + 2 * H * M
    NR = R // MC
    NSLOT = HG * NR * 2

    SA = 0
    SW = SA + NB
    SS = SW + NGT
    SX = SS + 1
    SOUT = SX + 1
    n_sems = SOUT + 1

    def kernel(x_hbm, k_hbm, v_hbm, sk_hbm, wq_hbm, wk_hbm, wv_hbm, wo_hbm,
               shift_hbm, dvec_hbm, gw_hbm, mem0_hbm, fwd_hbm, inv_hbm,
               out_hbm,
               x_v, wqkv, ar, gm, shift_ref, dvec_ref, gw_ref, mem0_ref, fwd_ref, inv_ref, sems):
        w_hbm = (wq_hbm, wk_hbm, wv_hbm)

        def wq_load(n, lo, hi):
            return pltpu.bitcast(wqkv[n, lo // 2:hi // 2, :], BF16)

        def wo_load(j, lo, hi):
            n, r = divmod(lo // 2, WROWS)
            return pltpu.bitcast(wqkv[3 * H + j * WPJ + n, r:r + (hi - lo) // 2, :], BF16)

        def rows(row, n, align):
            return pl.ds(row if isinstance(row, int) else pl.multiple_of(row, align), n)

        def ld_f32(row, n, align):
            return lax.bitcast_convert_type(ar[rows(row, n, align), :], F32)

        def st_f32(row, val, align):
            ar[rows(row, val.shape[0], align), :] = lax.bitcast_convert_type(val, U32)

        def ld_bf(row, n, align):
            return pltpu.bitcast(ar[rows(row, n, align), :], BF16)

        def st_bf(row, val, align):
            ar[rows(row, val.shape[0] // 2, align), :] = pltpu.bitcast(val, U32)

        cp_x = pltpu.make_async_copy(x_hbm, x_v, sems.at[SX])

        def prologue(k_v, v_v, sk_v, wst, wo_b, xp, xpu, dv_s):
            def cp_a(c):
                sl = c % ARING
                return [
                    pltpu.make_async_copy(k_hbm.at[:, pl.ds(c * LANES, LANES)], k_v.at[sl, pl.ds(KOFS, S), :],
                                          sems.at[SA + c]),
                    pltpu.make_async_copy(v_hbm.at[:, pl.ds(c * LANES, LANES)], v_v.at[sl], sems.at[SA + c]),
                    pltpu.make_async_copy(sk_hbm.at[pl.ds(c * LANES, LANES), :], sk_v.at[sl], sems.at[SA + c]),
                ]

            def cp_wo(j):
                return pltpu.make_async_copy(wo_hbm.at[:, pl.ds(j * LANES, LANES)], wo_b.at[j], sems.at[SA + j])

            def cp_w(gi):
                return pltpu.make_async_copy(w_hbm[gi // NG].at[:, pl.ds((gi % NG) * HG, HG), :], wst.at[gi],
                                             sems.at[SW + gi])

            def wait_w(gi):
                pltpu.make_async_copy(wst.at[gi], wst.at[gi], sems.at[SW + gi]).wait()

            small = [pltpu.make_async_copy(x_hbm.at[pl.ds(s * SEG, M), :], xp.at[pl.ds(s * M, M), :], sems.at[SS])
                     for s in range(NSEG)]
            small += [pltpu.make_async_copy(src, dst, sems.at[SS]) for src, dst in (
                (shift_hbm, shift_ref), (dvec_hbm, dvec_ref), (gw_hbm, gw_ref), (mem0_hbm, mem0_ref),
                (fwd_hbm, fwd_ref), (inv_hbm, inv_ref))]

            late = []
            for gi in range(1, NGT):
                late.append(cp_w(gi))
                c = gi - 1 - NP1
                if 0 <= c < ARING:
                    late += cp_a(c) + [cp_wo(c)]

            cp_w(0).start()
            for cp in small + late[:2]:
                cp.start()

            for c in range(ARING):
                k_v[c, KOFS - KPAD:KOFS, :] = jnp.zeros((KPAD, LANES), BF16)

            def dft_unit(c, j):
                sl = c % ARING
                r0 = j * CH
                sh = shift_ref[c].astype(F32)
                kw = k_v[sl, r0 + KOFS - KPAD:r0 + KOFS + CH, :].astype(F32)
                ks = kw[KPAD:] * sh[0:1, :]
                for t in range(1, KS):
                    ks = ks + kw[KPAD - t:KPAD - t + CH] * sh[t:t + 1, :]
                kv = (ks * v_v[sl, r0:r0 + CH, :].astype(F32)).astype(BF16)
                skc = sk_v[sl, :, r0:r0 + CH]
                off = (c * NC + j) * 2 * CH
                st_f32(UOFF + off, _dot(fwd_ref[0:CH, :], kv), CH)
                st_f32(UOFF + off + CH, _dot(fwd_ref[CH:, :], kv), CH)
                kr = _dot_nt(fwd_ref[0:CH, :], skc)
                if j == 0:
                    kr = kr + dv_s[pl.ds(c, 1), :]
                st_f32(KOFF + off, kr, CH)
                st_f32(KOFF + off + CH, _dot_nt(fwd_ref[CH:, :], skc), CH)

            def repack_blk(gi, i):
                blk = wst[gi, rows(i * 16, 16, 16)]
                wqkv[pl.ds(gi * HG, HG), rows(i * 8, 8, 8), :] = pltpu.bitcast(jnp.swapaxes(blk, 0, 1), U32)

            cp_w(0).wait()

            def rp0_body(i, c):
                repack_blk(0, i)
                return c
            lax.fori_loop(0, D // 16, rp0_body, 0, unroll=4)

            for cp in late[2:]:
                cp.start()
            for cp in small:
                cp.wait()
            dv_s[...] = dvec_ref[...].astype(F32)

            def xp_body(i, c):
                xr = xp[pl.ds(pl.multiple_of(i * 32, 32), 32), :]
                for kt in range(NB):
                    xpu[kt, pl.ds(pl.multiple_of(i * 16, 16), 16), :] = pltpu.bitcast(
                        xr[:, kt * LANES:(kt + 1) * LANES], U32)
                return c
            lax.fori_loop(0, R // 32, xp_body, 0)

            def pro_body(with_dft, it, c):
                nxt = jnp.minimum(it + 1, NGT - 1)
                rp0 = 0 if with_dft else NSLOT // 2
                upos = [lo for lo, _ in _split(NSLOT, NC)] if with_dft else []
                rslots = [t for t in range(rp0, NSLOT) if t not in upos and t - 1 not in upos]
                rp = dict(zip(rslots, _split(D // 16, len(rslots))))
                wr = H * E // NSLOT
                if with_dft:
                    cb = it - NP1
                    for cp in cp_a(cb) + [cp_wo(cb)]:
                        cp.wait()
                acc = None
                for sl in range(NSLOT):
                    hh, r, kk = sl // (2 * NR), (sl // 2) % NR, sl % 2
                    n = it * HG + hh
                    if sl == rp0:
                        @pl.when(it + 1 < NGT)
                        def _():
                            wait_w(it + 1)
                    if with_dft and sl == 1:
                        @pl.when((cb >= 1) & (cb <= NB - ARING))
                        def _():
                            xr = S // (NB - ARING)
                            x0 = pl.multiple_of((cb - 1) * xr, xr)
                            for cp in cp_a(cb - 1 + ARING) + [cp_wo(cb - 1 + ARING)]:
                                cp.start()
                            pltpu.make_async_copy(x_hbm.at[pl.ds(x0, xr), :], x_v.at[pl.ds(x0, xr), :],
                                                  sems.at[SX]).start()
                    for kt in range(kk * NB // 2, (kk + 1) * NB // 2):
                        lhs = pltpu.bitcast(xpu[kt, r * (MC // 2):(r + 1) * (MC // 2), :], BF16)
                        d = _dot(lhs, wq_load(n, kt * LANES, (kt + 1) * LANES))
                        acc = d if acc is None else d + acc
                    if kk == 1:
                        st_bf(n * (R // 2) + r * (MC // 2), acc.astype(BF16), MC // 2)
                        acc = None
                    if sl in rp:
                        for i in range(*rp[sl]):
                            repack_blk(nxt, i)
                    if with_dft:
                        n2, r2 = divmod(sl * wr // 2, WROWS)
                        wqkv[3 * H + cb * WPJ + n2, r2:r2 + wr // 2, :] = pltpu.bitcast(
                            wo_b[cb, sl * wr:(sl + 1) * wr, :], U32)
                    if sl in upos:
                        dft_unit(cb, upos.index(sl))
                return c
            lax.fori_loop(0, NP1, functools.partial(pro_body, False), 0)
            lax.fori_loop(NP1, NGT, functools.partial(pro_body, True), 0)

        pl.run_scoped(
            prologue,
            pltpu.VMEM((ARING, S + KOFS, LANES), BF16),
            pltpu.VMEM((ARING, S, LANES), BF16),
            pltpu.VMEM((ARING, LANES, S), BF16),
            pltpu.VMEM((NGT, D, HG, E), BF16),
            pltpu.VMEM((NB, H * E, LANES), BF16),
            pltpu.VMEM((R, D), BF16),
            pltpu.VMEM((NB, R // 2, LANES), U32),
            pltpu.VMEM((NB, LANES), F32),
        )

        def main(outb):
            cp_x.wait()

            def cp_out(q, lo, hi):
                nrow = EPI_SEGS * SEG
                r0 = pl.multiple_of(q * nrow, nrow)
                return pltpu.make_async_copy(outb.at[pl.ds(r0, nrow), pl.ds(lo, hi - lo)],
                                             out_hbm.at[pl.ds(r0, nrow), pl.ds(lo, hi - lo)], sems.at[SOUT])

            mac_steps = [(i0, j) for i0 in range(NC - MB, -1, -MB) for j in range(i0 + MB)]
            cum = np.cumsum([0] + [sum(1 for i in range(i0, i0 + MB) if i >= j) for i0, j in mac_steps])

            def make_mac(p, par, nparts):
                dyn = pl.multiple_of((p // (SPB // 2)) * NC * 2 * CH + (p % (SPB // 2)) * 2 * PR, 2 * PR)
                base = par * PR
                acc = {}
                kc = {}

                def ld(off):
                    return lax.bitcast_convert_type(ar[pl.ds(dyn + off, PR), :], F32)

                def run(lo, hi):
                    for (i0, j) in mac_steps[lo:hi]:
                        if j == 0:
                            kc.clear()
                        ur = ld(UOFF + base + j * 2 * CH)
                        ui = ld(UOFF + base + j * 2 * CH + CH)
                        for i in range(max(i0, j), i0 + MB):
                            m = i - j
                            if m not in kc:
                                kc[m] = (ld(KOFF + base + m * 2 * CH), ld(KOFF + base + m * 2 * CH + CH))
                            kr, ki = kc[m]
                            tr = ur * kr - ui * ki
                            ti = ur * ki + ui * kr
                            acc[i] = (tr, ti) if j == 0 else (acc[i][0] + tr, acc[i][1] + ti)
                        if j == i0 + MB - 1:
                            for i in range(i0, i0 + MB):
                                yr, yi = acc.pop(i)
                                row = dyn + UOFF + base + i * 2 * CH
                                ar[pl.ds(row, PR), :] = lax.bitcast_convert_type(yr, U32)
                                ar[pl.ds(row + CH, PR), :] = lax.bitcast_convert_type(yi, U32)
                cuts = [int(np.searchsorted(cum, cum[-1] * t / nparts)) for t in range(nparts)] + [len(mac_steps)]
                return [functools.partial(run, cuts[t], cuts[t + 1]) for t in range(nparts)]

            def masks(par):
                nq = SEG + 2 * M * par
                nk = SEG + 2 * M + 2 * M * par
                ri = lax.broadcasted_iota(jnp.int32, (nq, nk), 0)
                ci = lax.broadcasted_iota(jnp.int32, (nq, nk), 1)
                off = SEG + M * par

                def pos(i):
                    return jnp.where(i < M, i, jnp.where(i < SEG, i + M, i - off + M))

                valid = (ci < SEG) | ((ci >= off) & (ci < off + M))
                allowed = valid & ((ri < M) | (pos(ri) >= pos(ci)))
                if par == 1:
                    other = (ri >= SEG) & (ri < SEG + M)
                    mine = jnp.logical_not(other)
                    mem_a = (ci >= SEG + 2 * M) & (ci < SEG + 3 * M)
                    xa_lo = (ci >= SEG) & (ci < SEG + M)
                    xa_hi = ci >= SEG + 3 * M
                    valid = (other & (mem_a | xa_lo | xa_hi)) | (mine & valid)
                    allowed = (other & (mem_a | (xa_lo & (ri >= ci)))) | (mine & allowed)
                fill = jnp.where(valid, NEG, -jnp.inf).astype(F32)
                return allowed, fill

            def pair_body(p, mem):
                gw = gw_ref[...].astype(F32)
                for par in range(2):
                    allowed, fill = masks(par)
                    mac = make_mac(p, par, 2 * H)
                    r0 = pl.multiple_of(p * 2 * SEG + par * SEG, SEG)
                    xin = x_v[pl.ds(r0, SEG), :].astype(F32)
                    lhs = jnp.concatenate([mem, xin[M:]], axis=0).astype(BF16)
                    zp = xin[:, 0:LANES] * gw[0:1, :]
                    for kt in range(1, NB):
                        zp = zp + xin[:, kt * LANES:(kt + 1) * LANES] * gw[kt:kt + 1, :]
                    z = jnp.sum(zp, axis=1, keepdims=True)
                    g = jnp.broadcast_to(1.0 / (1.0 + jnp.exp(-z)), (SEG, LANES))
                    gm[pl.ds(r0, SEG), :] = g
                    o_in = [None] * H
                    qkv = {}
                    prob = {}

                    first = {(h, m): _dot(lhs[:, :D // 2], wq_load(m * H + h, 0, D // 2))
                             for h in range(KSPL) for m in range(3)}

                    def do_qkv(h):
                        out = []
                        for m in range(3):
                            if (h, m) in first:
                                t = _dot(lhs[:, D // 2:], wq_load(m * H + h, D // 2, D)) + first[(h, m)]
                            else:
                                t = _dot(lhs, wq_load(m * H + h, 0, D))
                            parts = [t]
                            if m > 0 or par == 1:
                                parts.append(ld_bf((m * H + h) * (R // 2) + p * M, M, M).astype(F32))
                            if m > 0:
                                sr = OOFF + (h * 2 + m - 1) * M
                                if par == 0:
                                    st_bf(sr, t[0:2 * M].astype(BF16), M)
                                else:
                                    parts.append(ld_bf(sr, M, M).astype(F32))
                                    st_f32(sr, t[0:M], M)
                                mac[2 * h + m - 1]()
                            out.append(jnp.concatenate(parts, axis=0).astype(BF16))
                        qkv[h] = out

                    def do_scores(h):
                        q, k, _ = qkv[h]
                        s = jnp.where(allowed, _dot_nt(q, k) * scale, fill)
                        e = jnp.exp(s - jnp.max(s, axis=1, keepdims=True))
                        l = jnp.sum(e, axis=1, keepdims=True)
                        prob[h] = (e * pl.reciprocal(l, approx=True)).astype(BF16)

                    def do_pv(h):
                        o = _dot(prob[h], qkv[h][2])
                        o_in[h] = o[0:SEG].astype(BF16)
                        if par == 1:
                            st_bf(h * (R // 2) + p * M, o[SEG:].astype(BF16), M)

                    def wo_part(j, h0, h1, acc):
                        for h in range(h0, h1):
                            t = _dot(o_in[h], wo_load(j, h * E, (h + 1) * E))
                            acc = t if acc is None else t + acc
                        return acc

                    res1 = []
                    for t in range(H // HP + LAG2):
                        for u in range(HP):
                            if t < H // HP:
                                do_qkv(t * HP + u)
                            elif len(res1) < NB:
                                res1.append(wo_part(len(res1), 0, KS_H, None))
                        if 0 <= t - LAG1 < H // HP:
                            for u in range(HP):
                                do_scores((t - LAG1) * HP + u)
                        if 0 <= t - LAG2 < H // HP:
                            for u in range(HP):
                                do_pv((t - LAG2) * HP + u)
                    while len(res1) < NB:
                        res1.append(wo_part(len(res1), 0, KS_H, None))
                    res = jnp.concatenate([wo_part(j, KS_H, H, res1[j]) for j in range(NB)], axis=1)
                    mem = res[0:M].astype(BF16).astype(F32)
                    g1 = jnp.concatenate([1.0 - g] * NB, axis=1)
                    outb[pl.ds(r0 + M, SEG - M), :] = (g1 * res)[M:].astype(BF16)
                return mem

            lax.fori_loop(0, NPAIR, pair_body, mem0_ref[...].astype(F32), unroll=2)

            ER = EPI_SEGS * M
            ROWS = EPI_SEGS * SEG

            def epi_body(q, c):
                r0 = pl.multiple_of(q * ROWS, ROWS)
                od = [ld_bf(h * (R // 2) + q * (ER // 2), ER // 2, ER // 2) for h in range(H)]
                iv = inv_ref[...]
                g = gm[pl.ds(r0, ROWS), :]
                for j in range(NB):
                    lo, hi = j * LANES, (j + 1) * LANES
                    res = None
                    for h in range(H):
                        t = _dot(od[h], wo_load(j, h * E, (h + 1) * E))
                        res = t if res is None else t + res
                    i0 = q * (ROWS // CH)
                    prev = ld_f32(UOFF + (j * NC + jnp.maximum(i0 - 1, 0)) * 2 * CH, 2 * CH, CH)
                    prev = jnp.where(i0 > 0, prev, 0.0)
                    ys = []
                    for i in range(ROWS // CH):
                        cur = ld_f32(UOFF + (j * NC + i0 + i) * 2 * CH, 2 * CH, CH)
                        z = jnp.concatenate([cur[0:HALF] - prev[CH:CH + HALF],
                                             cur[HALF:CH] + prev[CH + HALF:],
                                             cur[CH:CH + HALF] + prev[0:HALF],
                                             cur[CH + HALF:] - prev[HALF:CH]], axis=0).astype(BF16)
                        ys.append(_dot(iv, z))
                        prev = cur
                    y = jnp.concatenate(ys, axis=0)
                    a = g * (x_v[pl.ds(r0, ROWS), lo:hi].astype(F32) * y)
                    parts = []
                    for sgm in range(EPI_SEGS):
                        s0 = sgm * SEG
                        parts.append((1.0 - g[s0:s0 + M]) * res[sgm * M:(sgm + 1) * M])
                        parts.append(outb[pl.ds(r0 + s0 + M, SEG - M), lo:hi].astype(F32))
                    outb[pl.ds(r0, ROWS), lo:hi] = (a + jnp.concatenate(parts, axis=0)).astype(BF16)
                    if (j + 1) % OUTJ == 0:
                        cp_out(q, hi - OUTJ * LANES, hi).start()
                return c
            lax.fori_loop(0, N_EPI, epi_body, 0, unroll=2)
            pltpu.make_async_copy(outb, out_hbm, sems.at[SOUT]).wait()

        pl.run_scoped(main, pltpu.VMEM((S, D), BF16))

    scratch = [
        pltpu.VMEM((S, D), BF16),
        pltpu.VMEM((3 * H + NB * WPJ, WROWS, LANES), U32),
        pltpu.VMEM((AROWS, LANES), U32),
        pltpu.VMEM((S, LANES), F32),
        pltpu.VMEM((NB, KS, LANES), BF16),
        pltpu.VMEM((NB, LANES), BF16),
        pltpu.VMEM((NB, LANES), BF16),
        pltpu.VMEM((M, D), BF16),
        pltpu.VMEM((2 * CH, CH), BF16),
        pltpu.VMEM((CH, 2 * CH), BF16),
        pltpu.SemaphoreType.DMA((n_sems,)),
    ]
    return kernel, scratch


@functools.partial(jax.jit, static_argnames=("B_seg_len",))
def pallas_gated_mix__ssm_conv_h3__memory_aug_recurrent_mem_tr__prompt_kernel(
    A_q: jax.Array,
    A_k: jax.Array,
    A_v: jax.Array,
    A_shift_k: jax.Array,
    A_ssm_k: jax.Array,
    A_ssm_D: jax.Array,
    B_x: jax.Array,
    B_mem0: jax.Array,
    B_Wq: jax.Array,
    B_Wk: jax.Array,
    B_Wv: jax.Array,
    B_Wo: jax.Array,
    B_seg_len: int,
    gate_w: jax.Array,
):
    B, S, D = A_q.shape
    assert B == 1
    H, E = B_Wq.shape[1], B_Wq.shape[2]
    M = B_mem0.shape[1]
    KS = A_shift_k.shape[1]
    NB = D // LANES
    kernel, scratch = _make_kernel(S, D, H, E, M, int(B_seg_len), KS)
    fwd, inv = _dft_mats()

    any_spec = pl.BlockSpec(memory_space=pl.ANY)
    out = pl.pallas_call(
        kernel,
        out_shape=jax.ShapeDtypeStruct((S, D), A_q.dtype),
        in_specs=[any_spec] * 14,
        out_specs=any_spec,
        scratch_shapes=scratch,
        compiler_params=pltpu.CompilerParams(vmem_limit_bytes=126 * 1024 * 1024,
                                             disable_bounds_checks=True,
                                             disable_semaphore_checks=True),
    )(
        A_q.reshape(S, D), A_k.reshape(S, D), A_v.reshape(S, D), A_ssm_k,
        B_Wq, B_Wk, B_Wv, B_Wo.reshape(H * E, D),
        A_shift_k.reshape(NB, LANES, KS).transpose(0, 2, 1), A_ssm_D.reshape(NB, LANES),
        gate_w.reshape(NB, LANES), B_mem0.reshape(M, D),
        jnp.asarray(fwd, dtype=BF16), jnp.asarray(inv, dtype=BF16),
    )
    return out.reshape(1, S, D)
```

```python
import functools

import numpy as np
import jax
import jax.numpy as jnp
from jax import lax
import jax.experimental.pallas as pl
import jax.experimental.pallas.tpu as pltpu

F32 = jnp.float32
BF16 = jnp.bfloat16
U32 = jnp.uint32

LANES = 128
CH = 128
PR = 16
MB = 2
NEG = -1000000000.0
KPAD = 16
KOFS = 64
HG = 8
MC = 128
HP = 2
LAG1 = 1
LAG2 = 2
KS_H = 24
KSPL = 2
OUTJ = 2
EPI_SEGS = 8
ARING = 4
NP0 = 2
NQ = 4
NP1 = 4


def _dft_mats():
    f = np.concatenate([np.arange(0, CH, 2), np.arange(1, CH, 2)])
    t = np.arange(CH)
    ang = np.pi * np.outer(2 * f + 1, t) / (2 * CH)
    fwd = np.concatenate([np.cos(ang), -np.sin(ang)], axis=0)
    inv = np.concatenate([np.cos(ang).T, -np.sin(ang).T], axis=1) / CH
    return fwd.astype(np.float32), inv.astype(np.float32)


def _dot(a, b):
    return jnp.dot(a, b, preferred_element_type=F32)


def _dot_nt(a, b):
    return lax.dot_general(a, b, (((1,), (1,)), ((), ())), preferred_element_type=F32)


def _split(n, parts):
    return [((n * t) // parts, (n * (t + 1)) // parts) for t in range(parts)]


def _make_kernel(S, D, H, E, M, SEG, KS):
    assert E == LANES and M == 8 and SEG == 32 and D % LANES == 0 and S % (4 * SEG) == 0
    assert KS - 1 <= KPAD and H % HG == 0 and H % HP == 0
    NB = D // LANES
    NC = S // CH
    NSEG = S // SEG
    NPAIR = NSEG // 2
    R = NSEG * M
    NG = H // HG
    NGT = 3 * NG
    scale = float(E) ** -0.5
    HALF = CH // 2
    N_EPI = NSEG // EPI_SEGS
    SPB = CH // PR
    assert NB * SPB == NSEG
    assert NP0 + 1 <= NG
    assert NGT - NP1 == NB
    WROWS = D // 2
    WPJ = H * E // D
    UOFF = 3 * H * (R // 2)
    KOFF = UOFF + NB * NC * 2 * CH
    OOFF = KOFF + NB * NC * 2 * CH
    AROWS = OOFF + 2 * H * M
    NR = R // MC
    NSLOT = HG * NR * 2

    SA = 0
    SW = SA + NB
    SS = SW + NGT
    SX = SS + 1
    SOUT = SX + 1
    SQ = SOUT + 1
    NPC = (NP0 + 1) * NQ
    n_sems = SQ + NPC

    def kernel(x_hbm, x3_hbm, k_hbm, v_hbm, sk_hbm, wq_hbm, wk_hbm, wv_hbm, wo_hbm,
               shift_hbm, dvec_hbm, gw_hbm, mem0_hbm, fwd_hbm, inv_hbm,
               out_hbm,
               x_v, wqkv, ar, gm, shift_ref, dvec_ref, gw_ref, mem0_ref, fwd_ref, inv_ref, sems):
        w_hbm = (wq_hbm, wk_hbm, wv_hbm)

        def wq_load(n, lo, hi):
            return pltpu.bitcast(wqkv[n, lo // 2:hi // 2, :], BF16)

        def wo_load(j, lo, hi):
            n, r = divmod(lo // 2, WROWS)
            return pltpu.bitcast(wqkv[3 * H + j * WPJ + n, r:r + (hi - lo) // 2, :], BF16)

        def rows(row, n, align):
            return pl.ds(row if isinstance(row, int) else pl.multiple_of(row, align), n)

        def ld_f32(row, n, align):
            return lax.bitcast_convert_type(ar[rows(row, n, align), :], F32)

        def st_f32(row, val, align):
            ar[rows(row, val.shape[0], align), :] = lax.bitcast_convert_type(val, U32)

        def ld_bf(row, n, align):
            return pltpu.bitcast(ar[rows(row, n, align), :], BF16)

        def st_bf(row, val, align):
            ar[rows(row, val.shape[0] // 2, align), :] = pltpu.bitcast(val, U32)

        cp_x = pltpu.make_async_copy(x_hbm, x_v, sems.at[SX])

        def prologue(k_v, v_v, sk_v, wst, wo_b, xp, xpu, dv_s):
            def cp_a(c):
                sl = c % ARING
                return [
                    pltpu.make_async_copy(k_hbm.at[:, pl.ds(c * LANES, LANES)], k_v.at[sl, pl.ds(KOFS, S), :],
                                          sems.at[SA + c]),
                    pltpu.make_async_copy(v_hbm.at[:, pl.ds(c * LANES, LANES)], v_v.at[sl], sems.at[SA + c]),
                    pltpu.make_async_copy(sk_hbm.at[pl.ds(c * LANES, LANES), :], sk_v.at[sl], sems.at[SA + c]),
                ]

            def cp_wo(j):
                return pltpu.make_async_copy(wo_hbm.at[:, pl.ds(j * LANES, LANES)], wo_b.at[j], sems.at[SA + j])

            def cp_w(gi):
                return pltpu.make_async_copy(w_hbm[gi // NG].at[:, pl.ds((gi % NG) * HG, HG), :], wst.at[gi],
                                             sems.at[SW + gi])

            def wait_w(gi):
                pltpu.make_async_copy(wst.at[gi], wst.at[gi], sems.at[SW + gi]).wait()

            DQ = D // NQ

            def cp_piece(q):
                d0 = (q % NQ) * DQ
                return pltpu.make_async_copy(wq_hbm.at[pl.ds(d0, DQ), pl.ds((q // NQ) * HG, HG), :],
                                             wst.at[q // NQ, pl.ds(d0, DQ)], sems.at[SQ + q])

            def cp_xq(q):
                return pltpu.make_async_copy(x3_hbm.at[:, pl.ds(0, M), pl.ds(q * DQ, DQ)],
                                             xp.at[:, :, pl.ds(q * DQ, DQ)], sems.at[SQ + q])

            small = [pltpu.make_async_copy(src, dst, sems.at[SS]) for src, dst in (
                (shift_hbm, shift_ref), (dvec_hbm, dvec_ref), (gw_hbm, gw_ref), (mem0_hbm, mem0_ref),
                (fwd_hbm, fwd_ref), (inv_hbm, inv_ref))]

            late = []
            for gi in range(NP0 + 1, NGT):
                late.append(cp_w(gi))
                c = gi - 1 - NP1
                if 0 <= c < ARING:
                    late += cp_a(c) + [cp_wo(c)]

            for q in range(NPC):
                if q < NQ:
                    cp_xq(q).start()
                cp_piece(q).start()
                if q == NQ - 1:
                    for cp in small:
                        cp.start()
            for cp in late:
                cp.start()

            for c in range(ARING):
                k_v[c, KOFS - KPAD:KOFS, :] = jnp.zeros((KPAD, LANES), BF16)

            def dft_unit(c, j):
                sl = c % ARING
                r0 = j * CH
                sh = shift_ref[c].astype(F32)
                kw = k_v[sl, r0 + KOFS - KPAD:r0 + KOFS + CH, :].astype(F32)
                ks = kw[KPAD:] * sh[0:1, :]
                for t in range(1, KS):
                    ks = ks + kw[KPAD - t:KPAD - t + CH] * sh[t:t + 1, :]
                kv = (ks * v_v[sl, r0:r0 + CH, :].astype(F32)).astype(BF16)
                skc = sk_v[sl, :, r0:r0 + CH]
                off = (c * NC + j) * 2 * CH
                st_f32(UOFF + off, _dot(fwd_ref[0:CH, :], kv), CH)
                st_f32(UOFF + off + CH, _dot(fwd_ref[CH:, :], kv), CH)
                kr = _dot_nt(fwd_ref[0:CH, :], skc)
                if j == 0:
                    kr = kr + dv_s[pl.ds(c, 1), :]
                st_f32(KOFF + off, kr, CH)
                st_f32(KOFF + off + CH, _dot_nt(fwd_ref[CH:, :], skc), CH)

            def repack_blk(gi, i):
                blk = wst[gi, rows(i * 16, 16, 16)]
                wqkv[pl.ds(gi * HG, HG), rows(i * 8, 8, 8), :] = pltpu.bitcast(jnp.swapaxes(blk, 0, 1), U32)

            BPQ = DQ // 16
            KPQ = DQ // LANES

            def xconv(q, sp):
                for t in range(KPQ):
                    l0 = q * DQ + t * LANES
                    if not isinstance(l0, int):
                        l0 = pl.multiple_of(l0, LANES)
                    pair = jnp.concatenate([xp[2 * sp, :, pl.ds(l0, LANES)].astype(F32),
                                            xp[2 * sp + 1, :, pl.ds(l0, LANES)].astype(F32)], axis=0)
                    xpu[q * KPQ + t, rows(sp * M, M, M), :] = pltpu.bitcast(pair.astype(BF16), U32)

            AOFF = OOFF - NP0 * HG * R

            def zero_body(i, c):
                st_f32(AOFF + i * MC, jnp.zeros((MC, LANES), F32), MC)
                return c
            lax.fori_loop(0, NP0 * HG * NR, zero_body, 0)

            cp_xq(0).wait()
            cp_piece(0).wait()

            def pre_body(i, c):
                repack_blk(0, i)
                xconv(0, 2 * i)
                xconv(0, 2 * i + 1)
                return c
            assert NPAIR == 2 * BPQ
            lax.fori_loop(0, BPQ, pre_body, 0, unroll=2)

            def step_body(s, c):
                g = s // NQ
                qd = s % NQ
                p1 = s + 1
                p2 = jnp.where(s + NQ > NP0 * NQ, s + NQ, p1)
                xq = jnp.minimum(p1, NQ - 1)
                cp_piece(p1).wait()

                @pl.when(p1 < NQ)
                def _():
                    cp_xq(p1).wait()

                @pl.when(p2 != p1)
                def _():
                    cp_piece(p2).wait()
                nsl = HG * NR
                for sl in range(nsl):
                    hh, r = sl // NR, sl % NR
                    n = g * HG + hh
                    arow = AOFF + n * R + r * MC
                    acc = ld_f32(arow, MC, MC)
                    for t in range(KPQ):
                        kt = qd * KPQ + t
                        lhs = pltpu.bitcast(xpu[kt, r * (MC // 2):(r + 1) * (MC // 2), :], BF16)
                        w = wqkv[n, pl.ds(pl.multiple_of(kt * (LANES // 2), LANES // 2), LANES // 2), :]
                        acc = _dot(lhs, pltpu.bitcast(w, BF16)) + acc
                    st_f32(arow, acc, MC)
                    if sl % 2 == 1:
                        for pc in (p1, p2):
                            repack_blk(pc // NQ, (pc % NQ) * BPQ + sl // 2)
                        xconv(xq, sl - 1)
                        xconv(xq, sl)
                return c
            assert HG * NR == 2 * BPQ == NPAIR and NP1 == 2 * NP0 and NSLOT // 2 == HG * NR
            lax.fori_loop(0, NP0 * NQ, step_body, 0)

            for cp in small:
                cp.wait()
            dv_s[...] = dvec_ref[...].astype(F32)

            def pro_body(with_dft, it, c):
                nxt = jnp.minimum(it + 1, NGT - 1)
                rp0 = 0 if with_dft else NSLOT // 2
                upos = [lo for lo, _ in _split(NSLOT, NC)] if with_dft else []
                rslots = [t for t in range(rp0, NSLOT) if t not in upos and t - 1 not in upos]
                rp = dict(zip(rslots, _split(D // 16, len(rslots))))
                wr = H * E // NSLOT
                if with_dft:
                    cb = it - NP1
                    for cp in cp_a(cb) + [cp_wo(cb)]:
                        cp.wait()
                acc = None
                for sl in range(NSLOT):
                    hh, r, kk = sl // (2 * NR), (sl // 2) % NR, sl % 2
                    n = it * HG + hh
                    if sl == rp0:
                        @pl.when(it + 1 < NGT)
                        def _():
                            wait_w(it + 1)
                    if with_dft and sl == 1:
                        @pl.when((cb >= 1) & (cb <= NB - ARING))
                        def _():
                            xr = S // (NB - ARING)
                            x0 = pl.multiple_of((cb - 1) * xr, xr)
                            for cp in cp_a(cb - 1 + ARING) + [cp_wo(cb - 1 + ARING)]:
                                cp.start()
                            pltpu.make_async_copy(x_hbm.at[pl.ds(x0, xr), :], x_v.at[pl.ds(x0, xr), :],
                                                  sems.at[SX]).start()
                    for kt in range(kk * NB // 2, (kk + 1) * NB // 2):
                        lhs = pltpu.bitcast(xpu[kt, r * (MC // 2):(r + 1) * (MC // 2), :], BF16)
                        d = _dot(lhs, wq_load(n, kt * LANES, (kt + 1) * LANES))
                        acc = d if acc is None else d + acc
                    if kk == 1:
                        st_bf(n * (R // 2) + r * (MC // 2), acc.astype(BF16), MC // 2)
                        acc = None
                    if sl in rp:
                        for i in range(*rp[sl]):
                            repack_blk(nxt, i)
                    if not with_dft and sl < rp0:
                        nr0 = (it - NP0) * HG * R + sl * MC
                        st_bf(nr0 // 2, ld_f32(AOFF + nr0, MC, MC).astype(BF16), MC // 2)
                    if with_dft:
                        n2, r2 = divmod(sl * wr // 2, WROWS)
                        wqkv[3 * H + cb * WPJ + n2, r2:r2 + wr // 2, :] = pltpu.bitcast(
                            wo_b[cb, sl * wr:(sl + 1) * wr, :], U32)
                    if sl in upos:
                        dft_unit(cb, upos.index(sl))
                return c
            lax.fori_loop(NP0, NP1, functools.partial(pro_body, False), 0)
            lax.fori_loop(NP1, NGT, functools.partial(pro_body, True), 0)

        pl.run_scoped(
            prologue,
            pltpu.VMEM((ARING, S + KOFS, LANES), BF16),
            pltpu.VMEM((ARING, S, LANES), BF16),
            pltpu.VMEM((ARING, LANES, S), BF16),
            pltpu.VMEM((NGT, D, HG, E), BF16),
            pltpu.VMEM((NB, H * E, LANES), BF16),
            pltpu.VMEM((NSEG, M, D), BF16),
            pltpu.VMEM((NB, R // 2, LANES), U32),
            pltpu.VMEM((NB, LANES), F32),
        )

        def main(outb):
            cp_x.wait()

            def cp_out(q, lo, hi):
                nrow = EPI_SEGS * SEG
                r0 = pl.multiple_of(q * nrow, nrow)
                return pltpu.make_async_copy(outb.at[pl.ds(r0, nrow), pl.ds(lo, hi - lo)],
                                             out_hbm.at[pl.ds(r0, nrow), pl.ds(lo, hi - lo)], sems.at[SOUT])

            mac_steps = [(i0, j) for i0 in range(NC - MB, -1, -MB) for j in range(i0 + MB)]
            cum = np.cumsum([0] + [sum(1 for i in range(i0, i0 + MB) if i >= j) for i0, j in mac_steps])

            def make_mac(p, par, nparts):
                dyn = pl.multiple_of((p // (SPB // 2)) * NC * 2 * CH + (p % (SPB // 2)) * 2 * PR, 2 * PR)
                base = par * PR
                acc = {}
                kc = {}

                def ld(off):
                    return lax.bitcast_convert_type(ar[pl.ds(dyn + off, PR), :], F32)

                def run(lo, hi):
                    for (i0, j) in mac_steps[lo:hi]:
                        if j == 0:
                            kc.clear()
                        ur = ld(UOFF + base + j * 2 * CH)
                        ui = ld(UOFF + base + j * 2 * CH + CH)
                        for i in range(max(i0, j), i0 + MB):
                            m = i - j
                            if m not in kc:
                                kc[m] = (ld(KOFF + base + m * 2 * CH), ld(KOFF + base + m * 2 * CH + CH))
                            kr, ki = kc[m]
                            tr = ur * kr - ui * ki
                            ti = ur * ki + ui * kr
                            acc[i] = (tr, ti) if j == 0 else (acc[i][0] + tr, acc[i][1] + ti)
                        if j == i0 + MB - 1:
                            for i in range(i0, i0 + MB):
                                yr, yi = acc.pop(i)
                                row = dyn + UOFF + base + i * 2 * CH
                                ar[pl.ds(row, PR), :] = lax.bitcast_convert_type(yr, U32)
                                ar[pl.ds(row + CH, PR), :] = lax.bitcast_convert_type(yi, U32)
                cuts = [int(np.searchsorted(cum, cum[-1] * t / nparts)) for t in range(nparts)] + [len(mac_steps)]
                return [functools.partial(run, cuts[t], cuts[t + 1]) for t in range(nparts)]

            def masks(par):
                nq = SEG + 2 * M * par
                nk = SEG + 2 * M + 2 * M * par
                ri = lax.broadcasted_iota(jnp.int32, (nq, nk), 0)
                ci = lax.broadcasted_iota(jnp.int32, (nq, nk), 1)
                off = SEG + M * par

                def pos(i):
                    return jnp.where(i < M, i, jnp.where(i < SEG, i + M, i - off + M))

                valid = (ci < SEG) | ((ci >= off) & (ci < off + M))
                allowed = valid & ((ri < M) | (pos(ri) >= pos(ci)))
                if par == 1:
                    other = (ri >= SEG) & (ri < SEG + M)
                    mine = jnp.logical_not(other)
                    mem_a = (ci >= SEG + 2 * M) & (ci < SEG + 3 * M)
                    xa_lo = (ci >= SEG) & (ci < SEG + M)
                    xa_hi = ci >= SEG + 3 * M
                    valid = (other & (mem_a | xa_lo | xa_hi)) | (mine & valid)
                    allowed = (other & (mem_a | (xa_lo & (ri >= ci)))) | (mine & allowed)
                fill = jnp.where(valid, NEG, -jnp.inf).astype(F32)
                return allowed, fill

            def pair_body(p, mem):
                gw = gw_ref[...].astype(F32)
                for par in range(2):
                    allowed, fill = masks(par)
                    mac = make_mac(p, par, 2 * H)
                    r0 = pl.multiple_of(p * 2 * SEG + par * SEG, SEG)
                    xin = x_v[pl.ds(r0, SEG), :].astype(F32)
                    lhs = jnp.concatenate([mem, xin[M:]], axis=0).astype(BF16)
                    zp = xin[:, 0:LANES] * gw[0:1, :]
                    for kt in range(1, NB):
                        zp = zp + xin[:, kt * LANES:(kt + 1) * LANES] * gw[kt:kt + 1, :]
                    z = jnp.sum(zp, axis=1, keepdims=True)
                    g = jnp.broadcast_to(1.0 / (1.0 + jnp.exp(-z)), (SEG, LANES))
                    gm[pl.ds(r0, SEG), :] = g
                    o_in = [None] * H
                    qkv = {}
                    prob = {}

                    first = {(h, m): _dot(lhs[:, :D // 2], wq_load(m * H + h, 0, D // 2))
                             for h in range(KSPL) for m in range(3)}

                    def do_qkv(h):
                        out = []
                        for m in range(3):
                            if (h, m) in first:
                                t = _dot(lhs[:, D // 2:], wq_load(m * H + h, D // 2, D)) + first[(h, m)]
                            else:
                                t = _dot(lhs, wq_load(m * H + h, 0, D))
                            parts = [t]
                            if m > 0 or par == 1:
                                parts.append(ld_bf((m * H + h) * (R // 2) + p * M, M, M).astype(F32))
                            if m > 0:
                                sr = OOFF + (h * 2 + m - 1) * M
                                if par == 0:
                                    st_bf(sr, t[0:2 * M].astype(BF16), M)
                                else:
                                    parts.append(ld_bf(sr, M, M).astype(F32))
                                    st_f32(sr, t[0:M], M)
                                mac[2 * h + m - 1]()
                            out.append(jnp.concatenate(parts, axis=0).astype(BF16))
                        qkv[h] = out

                    def do_scores(h):
                        q, k, _ = qkv[h]
                        s = jnp.where(allowed, _dot_nt(q, k) * scale, fill)
                        e = jnp.exp(s - jnp.max(s, axis=1, keepdims=True))
                        l = jnp.sum(e, axis=1, keepdims=True)
                        prob[h] = (e * pl.reciprocal(l, approx=True)).astype(BF16)

                    def do_pv(h):
                        o = _dot(prob[h], qkv[h][2])
                        o_in[h] = o[0:SEG].astype(BF16)
                        if par == 1:
                            st_bf(h * (R // 2) + p * M, o[SEG:].astype(BF16), M)

                    def wo_part(j, h0, h1, acc):
                        for h in range(h0, h1):
                            t = _dot(o_in[h], wo_load(j, h * E, (h + 1) * E))
                            acc = t if acc is None else t + acc
                        return acc

                    res1 = []
                    for t in range(H // HP + LAG2):
                        for u in range(HP):
                            if t < H // HP:
                                do_qkv(t * HP + u)
                            elif len(res1) < NB:
                                res1.append(wo_part(len(res1), 0, KS_H, None))
                        if 0 <= t - LAG1 < H // HP:
                            for u in range(HP):
                                do_scores((t - LAG1) * HP + u)
                        if 0 <= t - LAG2 < H // HP:
                            for u in range(HP):
                                do_pv((t - LAG2) * HP + u)
                    while len(res1) < NB:
                        res1.append(wo_part(len(res1), 0, KS_H, None))
                    res = jnp.concatenate([wo_part(j, KS_H, H, res1[j]) for j in range(NB)], axis=1)
                    mem = res[0:M].astype(BF16).astype(F32)
                    g1 = jnp.concatenate([1.0 - g] * NB, axis=1)
                    outb[pl.ds(r0 + M, SEG - M), :] = (g1 * res)[M:].astype(BF16)
                return mem

            lax.fori_loop(0, NPAIR, pair_body, mem0_ref[...].astype(F32), unroll=2)

            ER = EPI_SEGS * M
            ROWS = EPI_SEGS * SEG

            def epi_body(q, c):
                r0 = pl.multiple_of(q * ROWS, ROWS)
                od = [ld_bf(h * (R // 2) + q * (ER // 2), ER // 2, ER // 2) for h in range(H)]
                iv = inv_ref[...]
                g = gm[pl.ds(r0, ROWS), :]
                for j in range(NB):
                    lo, hi = j * LANES, (j + 1) * LANES
                    res = None
                    for h in range(H):
                        t = _dot(od[h], wo_load(j, h * E, (h + 1) * E))
                        res = t if res is None else t + res
                    i0 = q * (ROWS // CH)
                    prev = ld_f32(UOFF + (j * NC + jnp.maximum(i0 - 1, 0)) * 2 * CH, 2 * CH, CH)
                    prev = jnp.where(i0 > 0, prev, 0.0)
                    ys = []
                    for i in range(ROWS // CH):
                        cur = ld_f32(UOFF + (j * NC + i0 + i) * 2 * CH, 2 * CH, CH)
                        z = jnp.concatenate([cur[0:HALF] - prev[CH:CH + HALF],
                                             cur[HALF:CH] + prev[CH + HALF:],
                                             cur[CH:CH + HALF] + prev[0:HALF],
                                             cur[CH + HALF:] - prev[HALF:CH]], axis=0).astype(BF16)
                        ys.append(_dot(iv, z))
                        prev = cur
                    y = jnp.concatenate(ys, axis=0)
                    a = g * (x_v[pl.ds(r0, ROWS), lo:hi].astype(F32) * y)
                    parts = []
                    for sgm in range(EPI_SEGS):
                        s0 = sgm * SEG
                        parts.append((1.0 - g[s0:s0 + M]) * res[sgm * M:(sgm + 1) * M])
                        parts.append(outb[pl.ds(r0 + s0 + M, SEG - M), lo:hi].astype(F32))
                    outb[pl.ds(r0, ROWS), lo:hi] = (a + jnp.concatenate(parts, axis=0)).astype(BF16)
                    if (j + 1) % OUTJ == 0:
                        cp_out(q, hi - OUTJ * LANES, hi).start()
                return c
            lax.fori_loop(0, N_EPI, epi_body, 0, unroll=2)
            pltpu.make_async_copy(outb, out_hbm, sems.at[SOUT]).wait()

        pl.run_scoped(main, pltpu.VMEM((S, D), BF16))

    scratch = [
        pltpu.VMEM((S, D), BF16),
        pltpu.VMEM((3 * H + NB * WPJ, WROWS, LANES), U32),
        pltpu.VMEM((AROWS, LANES), U32),
        pltpu.VMEM((S, LANES), F32),
        pltpu.VMEM((NB, KS, LANES), BF16),
        pltpu.VMEM((NB, LANES), BF16),
        pltpu.VMEM((NB, LANES), BF16),
        pltpu.VMEM((M, D), BF16),
        pltpu.VMEM((2 * CH, CH), BF16),
        pltpu.VMEM((CH, 2 * CH), BF16),
        pltpu.SemaphoreType.DMA((n_sems,)),
    ]
    return kernel, scratch


@functools.partial(jax.jit, static_argnames=("B_seg_len",))
def pallas_gated_mix__ssm_conv_h3__memory_aug_recurrent_mem_tr__prompt_kernel(
    A_q: jax.Array,
    A_k: jax.Array,
    A_v: jax.Array,
    A_shift_k: jax.Array,
    A_ssm_k: jax.Array,
    A_ssm_D: jax.Array,
    B_x: jax.Array,
    B_mem0: jax.Array,
    B_Wq: jax.Array,
    B_Wk: jax.Array,
    B_Wv: jax.Array,
    B_Wo: jax.Array,
    B_seg_len: int,
    gate_w: jax.Array,
):
    B, S, D = A_q.shape
    assert B == 1
    H, E = B_Wq.shape[1], B_Wq.shape[2]
    M = B_mem0.shape[1]
    KS = A_shift_k.shape[1]
    NB = D // LANES
    kernel, scratch = _make_kernel(S, D, H, E, M, int(B_seg_len), KS)
    fwd, inv = _dft_mats()

    any_spec = pl.BlockSpec(memory_space=pl.ANY)
    out = pl.pallas_call(
        kernel,
        out_shape=jax.ShapeDtypeStruct((S, D), A_q.dtype),
        in_specs=[any_spec] * 15,
        out_specs=any_spec,
        scratch_shapes=scratch,
        compiler_params=pltpu.CompilerParams(vmem_limit_bytes=126 * 1024 * 1024,
                                             disable_bounds_checks=True,
                                             disable_semaphore_checks=True),
    )(
        A_q.reshape(S, D), A_q.reshape(S // int(B_seg_len), int(B_seg_len), D), A_k.reshape(S, D), A_v.reshape(S, D), A_ssm_k,
        B_Wq, B_Wk, B_Wv, B_Wo.reshape(H * E, D),
        A_shift_k.reshape(NB, LANES, KS).transpose(0, 2, 1), A_ssm_D.reshape(NB, LANES),
        gate_w.reshape(NB, LANES), B_mem0.reshape(M, D),
        jnp.asarray(fwd, dtype=BF16), jnp.asarray(inv, dtype=BF16),
    )
    return out.reshape(1, S, D)
```

```python
import functools

import numpy as np
import jax
import jax.numpy as jnp
from jax import lax
import jax.experimental.pallas as pl
import jax.experimental.pallas.tpu as pltpu

F32 = jnp.float32
BF16 = jnp.bfloat16
U32 = jnp.uint32

LANES = 128
CH = 128
PR = 16
MB = 2
NEG = -1000000000.0
KPAD = 16
KOFS = 64
HG = 8
MC = 128
HP = 2
LAG1 = 1
LAG2 = 2
KS_H = 24
KSPL = 2
OUTJ = 2
EPI_SEGS = 8
ARING = 4
NP0 = 2
NQ = 4
NP1 = 4


def _dft_mats():
    f = np.concatenate([np.arange(0, CH, 2), np.arange(1, CH, 2)])
    th = np.pi * (2 * f + 1) / (2 * CH)
    t = np.arange(CH)
    ang_u = np.outer(th, t + 0.5)
    ang_k = np.outer(th, t)
    fwd = np.stack([np.concatenate([np.cos(a), -np.sin(a)], axis=0) for a in (ang_u, ang_k)])
    ph = ang_u.T[:CH // 2]
    cps, cms = np.cos(ph) + np.sin(ph), np.cos(ph) - np.sin(ph)
    even = np.arange(CH) < CH // 2
    inv = np.stack([np.where(even, cps, cms), np.where(even, cms, cps)]) / (2 * CH)
    return fwd.astype(np.float32), inv.astype(np.float32)


def _flip_rows(v):
    i = lax.broadcasted_iota(jnp.int32, (8, LANES), 0)
    out = []
    for t in range(v.shape[0] // 8 - 1, -1, -1):
        w = pltpu.roll(v[8 * t:8 * t + 8], 4, 0)
        w = jnp.where((i & 2) == 0, pltpu.roll(w, 6, 0), pltpu.roll(w, 2, 0))
        out.append(jnp.where((i & 1) == 0, pltpu.roll(w, 7, 0), pltpu.roll(w, 1, 0)))
    return jnp.concatenate(out, axis=0)


def _dot(a, b):
    return jnp.dot(a, b, preferred_element_type=F32)


def _dot_nt(a, b):
    return lax.dot_general(a, b, (((1,), (1,)), ((), ())), preferred_element_type=F32)


def _split(n, parts):
    return [((n * t) // parts, (n * (t + 1)) // parts) for t in range(parts)]


def _make_kernel(S, D, H, E, M, SEG, KS):
    assert E == LANES and M == 8 and SEG == 32 and D % LANES == 0 and S % (4 * SEG) == 0
    assert KS - 1 <= KPAD and H % HG == 0 and H % HP == 0
    NB = D // LANES
    NC = S // CH
    NSEG = S // SEG
    NPAIR = NSEG // 2
    R = NSEG * M
    NG = H // HG
    NGT = 3 * NG
    scale = float(E) ** -0.5
    HALF = CH // 2
    N_EPI = NSEG // EPI_SEGS
    SPB = CH // PR
    assert NB * SPB == NSEG
    assert NP0 + 1 <= NG
    assert NGT - NP1 == NB
    WROWS = D // 2
    WPJ = H * E // D
    UOFF = 3 * H * (R // 2)
    KOFF = UOFF + NB * NC * 2 * CH
    OOFF = KOFF + NB * NC * 2 * CH
    AROWS = OOFF + 2 * H * M
    NR = R // MC
    NSLOT = HG * NR * 2

    SA = 0
    SW = SA + NB
    SS = SW + NGT
    SX = SS + 1
    SOUT = SX + 1
    SQ = SOUT + 1
    NPC = (NP0 + 1) * NQ
    n_sems = SQ + NPC

    def kernel(x_hbm, x3_hbm, k_hbm, v_hbm, sk_hbm, wq_hbm, wk_hbm, wv_hbm, wo_hbm,
               shift_hbm, dvec_hbm, gw_hbm, mem0_hbm, fwd_hbm, inv_hbm,
               out_hbm,
               x_v, wqkv, ar, gm, shift_ref, dvec_ref, gw_ref, mem0_ref, fwd_ref, inv_ref, sems):
        w_hbm = (wq_hbm, wk_hbm, wv_hbm)

        def wq_load(n, lo, hi):
            return pltpu.bitcast(wqkv[n, lo // 2:hi // 2, :], BF16)

        def wo_load(j, lo, hi):
            n, r = divmod(lo // 2, WROWS)
            return pltpu.bitcast(wqkv[3 * H + j * WPJ + n, r:r + (hi - lo) // 2, :], BF16)

        def rows(row, n, align):
            return pl.ds(row if isinstance(row, int) else pl.multiple_of(row, align), n)

        def ld_f32(row, n, align):
            return lax.bitcast_convert_type(ar[rows(row, n, align), :], F32)

        def st_f32(row, val, align):
            ar[rows(row, val.shape[0], align), :] = lax.bitcast_convert_type(val, U32)

        def ld_bf(row, n, align):
            return pltpu.bitcast(ar[rows(row, n, align), :], BF16)

        def st_bf(row, val, align):
            ar[rows(row, val.shape[0] // 2, align), :] = pltpu.bitcast(val, U32)

        cp_x = pltpu.make_async_copy(x_hbm, x_v, sems.at[SX])

        def prologue(k_v, v_v, sk_v, wst, wo_b, xp, xpu, dv_s):
            def cp_a(c):
                sl = c % ARING
                return [
                    pltpu.make_async_copy(k_hbm.at[:, pl.ds(c * LANES, LANES)], k_v.at[sl, pl.ds(KOFS, S), :],
                                          sems.at[SA + c]),
                    pltpu.make_async_copy(v_hbm.at[:, pl.ds(c * LANES, LANES)], v_v.at[sl], sems.at[SA + c]),
                    pltpu.make_async_copy(sk_hbm.at[pl.ds(c * LANES, LANES), :], sk_v.at[sl], sems.at[SA + c]),
                ]

            def cp_wo(j):
                return pltpu.make_async_copy(wo_hbm.at[:, pl.ds(j * LANES, LANES)], wo_b.at[j], sems.at[SA + j])

            def cp_w(gi):
                return pltpu.make_async_copy(w_hbm[gi // NG].at[:, pl.ds((gi % NG) * HG, HG), :], wst.at[gi],
                                             sems.at[SW + gi])

            def wait_w(gi):
                pltpu.make_async_copy(wst.at[gi], wst.at[gi], sems.at[SW + gi]).wait()

            DQ = D // NQ

            def cp_piece(q):
                d0 = (q % NQ) * DQ
                return pltpu.make_async_copy(wq_hbm.at[pl.ds(d0, DQ), pl.ds((q // NQ) * HG, HG), :],
                                             wst.at[q // NQ, pl.ds(d0, DQ)], sems.at[SQ + q])

            def cp_xq(q):
                return pltpu.make_async_copy(x3_hbm.at[:, pl.ds(0, M), pl.ds(q * DQ, DQ)],
                                             xp.at[:, :, pl.ds(q * DQ, DQ)], sems.at[SQ + q])

            small = [pltpu.make_async_copy(src, dst, sems.at[SS]) for src, dst in (
                (shift_hbm, shift_ref), (dvec_hbm, dvec_ref), (gw_hbm, gw_ref), (mem0_hbm, mem0_ref),
                (fwd_hbm, fwd_ref), (inv_hbm, inv_ref))]

            late = []
            for gi in range(NP0 + 1, NGT):
                late.append(cp_w(gi))
                c = gi - 1 - NP1
                if 0 <= c < ARING:
                    late += cp_a(c) + [cp_wo(c)]

            for q in range(NPC):
                if q < NQ:
                    cp_xq(q).start()
                cp_piece(q).start()
                if q == NQ - 1:
                    for cp in small:
                        cp.start()
            for cp in late:
                cp.start()

            for c in range(ARING):
                k_v[c, KOFS - KPAD:KOFS, :] = jnp.zeros((KPAD, LANES), BF16)

            def dft_unit(c, j):
                sl = c % ARING
                r0 = j * CH
                sh = shift_ref[c].astype(F32)
                kw = k_v[sl, r0 + KOFS - KPAD:r0 + KOFS + CH, :].astype(F32)
                ks = kw[KPAD:] * sh[0:1, :]
                for t in range(1, KS):
                    ks = ks + kw[KPAD - t:KPAD - t + CH] * sh[t:t + 1, :]
                kv = (ks * v_v[sl, r0:r0 + CH, :].astype(F32)).astype(BF16)
                skc = sk_v[sl, :, r0:r0 + CH]
                off = (c * NC + j) * 2 * CH
                st_f32(UOFF + off, _dot(fwd_ref[0, 0:CH, :], kv), CH)
                st_f32(UOFF + off + CH, _dot(fwd_ref[0, CH:, :], kv), CH)
                kr = _dot_nt(fwd_ref[1, 0:CH, :], skc)
                if j == 0:
                    kr = kr + dv_s[pl.ds(c, 1), :]
                st_f32(KOFF + off, kr, CH)
                st_f32(KOFF + off + CH, _dot_nt(fwd_ref[1, CH:, :], skc), CH)

            def repack_blk(gi, i):
                blk = wst[gi, rows(i * 16, 16, 16)]
                wqkv[pl.ds(gi * HG, HG), rows(i * 8, 8, 8), :] = pltpu.bitcast(jnp.swapaxes(blk, 0, 1), U32)

            BPQ = DQ // 16
            KPQ = DQ // LANES

            def xconv(q, sp):
                for t in range(KPQ):
                    l0 = q * DQ + t * LANES
                    if not isinstance(l0, int):
                        l0 = pl.multiple_of(l0, LANES)
                    pair = jnp.concatenate([xp[2 * sp, :, pl.ds(l0, LANES)].astype(F32),
                                            xp[2 * sp + 1, :, pl.ds(l0, LANES)].astype(F32)], axis=0)
                    xpu[q * KPQ + t, rows(sp * M, M, M), :] = pltpu.bitcast(pair.astype(BF16), U32)

            AOFF = OOFF - NP0 * HG * R

            def zero_body(i, c):
                st_f32(AOFF + i * MC, jnp.zeros((MC, LANES), F32), MC)
                return c
            lax.fori_loop(0, NP0 * HG * NR, zero_body, 0)

            cp_xq(0).wait()
            cp_piece(0).wait()

            def pre_body(i, c):
                repack_blk(0, i)
                xconv(0, 2 * i)
                xconv(0, 2 * i + 1)
                return c
            assert NPAIR == 2 * BPQ
            lax.fori_loop(0, BPQ, pre_body, 0, unroll=2)

            def step_body(s, c):
                g = s // NQ
                qd = s % NQ
                p1 = s + 1
                p2 = jnp.where(s + NQ > NP0 * NQ, s + NQ, p1)
                xq = jnp.minimum(p1, NQ - 1)
                cp_piece(p1).wait()

                @pl.when(p1 < NQ)
                def _():
                    cp_xq(p1).wait()

                @pl.when(p2 != p1)
                def _():
                    cp_piece(p2).wait()
                nsl = HG * NR
                for sl in range(nsl):
                    hh, r = sl // NR, sl % NR
                    n = g * HG + hh
                    arow = AOFF + n * R + r * MC
                    acc = ld_f32(arow, MC, MC)
                    for t in range(KPQ):
                        kt = qd * KPQ + t
                        lhs = pltpu.bitcast(xpu[kt, r * (MC // 2):(r + 1) * (MC // 2), :], BF16)
                        w = wqkv[n, pl.ds(pl.multiple_of(kt * (LANES // 2), LANES // 2), LANES // 2), :]
                        acc = _dot(lhs, pltpu.bitcast(w, BF16)) + acc
                    st_f32(arow, acc, MC)
                    if sl % 2 == 1:
                        for pc in (p1, p2):
                            repack_blk(pc // NQ, (pc % NQ) * BPQ + sl // 2)
                        xconv(xq, sl - 1)
                        xconv(xq, sl)
                return c
            assert HG * NR == 2 * BPQ == NPAIR and NP1 == 2 * NP0 and NSLOT // 2 == HG * NR
            lax.fori_loop(0, NP0 * NQ, step_body, 0)

            for cp in small:
                cp.wait()
            dv_s[...] = dvec_ref[...].astype(F32)

            def pro_body(with_dft, it, c):
                nxt = jnp.minimum(it + 1, NGT - 1)
                rp0 = 0 if with_dft else NSLOT // 2
                upos = [lo for lo, _ in _split(NSLOT, NC)] if with_dft else []
                rslots = [t for t in range(rp0, NSLOT) if t not in upos and t - 1 not in upos]
                rp = dict(zip(rslots, _split(D // 16, len(rslots))))
                wr = H * E // NSLOT
                if with_dft:
                    cb = it - NP1
                    for cp in cp_a(cb) + [cp_wo(cb)]:
                        cp.wait()
                acc = None
                for sl in range(NSLOT):
                    hh, r, kk = sl // (2 * NR), (sl // 2) % NR, sl % 2
                    n = it * HG + hh
                    if sl == rp0:
                        @pl.when(it + 1 < NGT)
                        def _():
                            wait_w(it + 1)
                    if with_dft and sl == 1:
                        @pl.when((cb >= 1) & (cb <= NB - ARING))
                        def _():
                            xr = S // (NB - ARING)
                            x0 = pl.multiple_of((cb - 1) * xr, xr)
                            for cp in cp_a(cb - 1 + ARING) + [cp_wo(cb - 1 + ARING)]:
                                cp.start()
                            pltpu.make_async_copy(x_hbm.at[pl.ds(x0, xr), :], x_v.at[pl.ds(x0, xr), :],
                                                  sems.at[SX]).start()
                    for kt in range(kk * NB // 2, (kk + 1) * NB // 2):
                        lhs = pltpu.bitcast(xpu[kt, r * (MC // 2):(r + 1) * (MC // 2), :], BF16)
                        d = _dot(lhs, wq_load(n, kt * LANES, (kt + 1) * LANES))
                        acc = d if acc is None else d + acc
                    if kk == 1:
                        st_bf(n * (R // 2) + r * (MC // 2), acc.astype(BF16), MC // 2)
                        acc = None
                    if sl in rp:
                        for i in range(*rp[sl]):
                            repack_blk(nxt, i)
                    if not with_dft and sl < rp0:
                        nr0 = (it - NP0) * HG * R + sl * MC
                        st_bf(nr0 // 2, ld_f32(AOFF + nr0, MC, MC).astype(BF16), MC // 2)
                    if with_dft:
                        n2, r2 = divmod(sl * wr // 2, WROWS)
                        wqkv[3 * H + cb * WPJ + n2, r2:r2 + wr // 2, :] = pltpu.bitcast(
                            wo_b[cb, sl * wr:(sl + 1) * wr, :], U32)
                    if sl in upos:
                        dft_unit(cb, upos.index(sl))
                return c
            lax.fori_loop(NP0, NP1, functools.partial(pro_body, False), 0)
            lax.fori_loop(NP1, NGT, functools.partial(pro_body, True), 0)

        pl.run_scoped(
            prologue,
            pltpu.VMEM((ARING, S + KOFS, LANES), BF16),
            pltpu.VMEM((ARING, S, LANES), BF16),
            pltpu.VMEM((ARING, LANES, S), BF16),
            pltpu.VMEM((NGT, D, HG, E), BF16),
            pltpu.VMEM((NB, H * E, LANES), BF16),
            pltpu.VMEM((NSEG, M, D), BF16),
            pltpu.VMEM((NB, R // 2, LANES), U32),
            pltpu.VMEM((NB, LANES), F32),
        )

        def main(outb):
            cp_x.wait()

            def cp_out(q, lo, hi):
                nrow = EPI_SEGS * SEG
                r0 = pl.multiple_of(q * nrow, nrow)
                return pltpu.make_async_copy(outb.at[pl.ds(r0, nrow), pl.ds(lo, hi - lo)],
                                             out_hbm.at[pl.ds(r0, nrow), pl.ds(lo, hi - lo)], sems.at[SOUT])

            mac_steps = [(i0, j) for i0 in range(NC - MB, -1, -MB) for j in range(i0 + MB)]
            cum = np.cumsum([0] + [sum(1 for i in range(i0, i0 + MB) if i >= j) for i0, j in mac_steps])

            def make_mac(p, par, nparts):
                dyn = pl.multiple_of((p // (SPB // 2)) * NC * 2 * CH + (p % (SPB // 2)) * 2 * PR, 2 * PR)
                base = par * PR
                acc = {}
                kc = {}

                def ld(off):
                    return lax.bitcast_convert_type(ar[pl.ds(dyn + off, PR), :], F32)

                def run(lo, hi):
                    for (i0, j) in mac_steps[lo:hi]:
                        if j == 0:
                            kc.clear()
                        ur = ld(UOFF + base + j * 2 * CH)
                        ui = ld(UOFF + base + j * 2 * CH + CH)
                        for i in range(max(i0, j), i0 + MB):
                            m = i - j
                            if m not in kc:
                                kc[m] = (ld(KOFF + base + m * 2 * CH), ld(KOFF + base + m * 2 * CH + CH))
                            kr, ki = kc[m]
                            tr = ur * kr - ui * ki
                            ti = ur * ki + ui * kr
                            acc[i] = (tr, ti) if j == 0 else (acc[i][0] + tr, acc[i][1] + ti)
                        if j == i0 + MB - 1:
                            for i in range(i0, i0 + MB):
                                yr, yi = acc.pop(i)
                                row = dyn + UOFF + base + i * 2 * CH
                                ar[pl.ds(row, PR), :] = lax.bitcast_convert_type(yr, U32)
                                ar[pl.ds(row + CH, PR), :] = lax.bitcast_convert_type(yi, U32)
                cuts = [int(np.searchsorted(cum, cum[-1] * t / nparts)) for t in range(nparts)] + [len(mac_steps)]
                return [functools.partial(run, cuts[t], cuts[t + 1]) for t in range(nparts)]

            def masks(par):
                nq = SEG + 2 * M * par
                nk = SEG + 2 * M + 2 * M * par
                ri = lax.broadcasted_iota(jnp.int32, (nq, nk), 0)
                ci = lax.broadcasted_iota(jnp.int32, (nq, nk), 1)
                off = SEG + M * par

                def pos(i):
                    return jnp.where(i < M, i, jnp.where(i < SEG, i + M, i - off + M))

                valid = (ci < SEG) | ((ci >= off) & (ci < off + M))
                allowed = valid & ((ri < M) | (pos(ri) >= pos(ci)))
                if par == 1:
                    other = (ri >= SEG) & (ri < SEG + M)
                    mine = jnp.logical_not(other)
                    mem_a = (ci >= SEG + 2 * M) & (ci < SEG + 3 * M)
                    xa_lo = (ci >= SEG) & (ci < SEG + M)
                    xa_hi = ci >= SEG + 3 * M
                    valid = (other & (mem_a | xa_lo | xa_hi)) | (mine & valid)
                    allowed = (other & (mem_a | (xa_lo & (ri >= ci)))) | (mine & allowed)
                fill = jnp.where(valid, NEG, -jnp.inf).astype(F32)
                return allowed, fill

            def pair_body(p, mem):
                gw = gw_ref[...].astype(F32)
                for par in range(2):
                    allowed, fill = masks(par)
                    mac = make_mac(p, par, 2 * H)
                    r0 = pl.multiple_of(p * 2 * SEG + par * SEG, SEG)
                    xin = x_v[pl.ds(r0, SEG), :].astype(F32)
                    lhs = jnp.concatenate([mem, xin[M:]], axis=0).astype(BF16)
                    zp = xin[:, 0:LANES] * gw[0:1, :]
                    for kt in range(1, NB):
                        zp = zp + xin[:, kt * LANES:(kt + 1) * LANES] * gw[kt:kt + 1, :]
                    z = jnp.sum(zp, axis=1, keepdims=True)
                    g = jnp.broadcast_to(1.0 / (1.0 + jnp.exp(-z)), (SEG, LANES))
                    gm[pl.ds(r0, SEG), :] = g
                    o_in = [None] * H
                    qkv = {}
                    prob = {}

                    first = {(h, m): _dot(lhs[:, :D // 2], wq_load(m * H + h, 0, D // 2))
                             for h in range(KSPL) for m in range(3)}

                    def do_qkv(h):
                        out = []
                        for m in range(3):
                            if (h, m) in first:
                                t = _dot(lhs[:, D // 2:], wq_load(m * H + h, D // 2, D)) + first[(h, m)]
                            else:
                                t = _dot(lhs, wq_load(m * H + h, 0, D))
                            parts = [t]
                            if m > 0 or par == 1:
                                parts.append(ld_bf((m * H + h) * (R // 2) + p * M, M, M).astype(F32))
                            if m > 0:
                                sr = OOFF + (h * 2 + m - 1) * M
                                if par == 0:
                                    st_bf(sr, t[0:2 * M].astype(BF16), M)
                                else:
                                    parts.append(ld_bf(sr, M, M).astype(F32))
                                    st_f32(sr, t[0:M], M)
                                mac[2 * h + m - 1]()
                            out.append(jnp.concatenate(parts, axis=0).astype(BF16))
                        qkv[h] = out

                    def do_scores(h):
                        q, k, _ = qkv[h]
                        s = jnp.where(allowed, _dot_nt(q, k) * scale, fill)
                        e = jnp.exp(s - jnp.max(s, axis=1, keepdims=True))
                        l = jnp.sum(e, axis=1, keepdims=True)
                        prob[h] = (e * pl.reciprocal(l, approx=True)).astype(BF16)

                    def do_pv(h):
                        o = _dot(prob[h], qkv[h][2])
                        o_in[h] = o[0:SEG].astype(BF16)
                        if par == 1:
                            st_bf(h * (R // 2) + p * M, o[SEG:].astype(BF16), M)

                    def wo_part(j, h0, h1, acc):
                        for h in range(h0, h1):
                            t = _dot(o_in[h], wo_load(j, h * E, (h + 1) * E))
                            acc = t if acc is None else t + acc
                        return acc

                    res1 = []
                    for t in range(H // HP + LAG2):
                        for u in range(HP):
                            if t < H // HP:
                                do_qkv(t * HP + u)
                            elif len(res1) < NB:
                                res1.append(wo_part(len(res1), 0, KS_H, None))
                        if 0 <= t - LAG1 < H // HP:
                            for u in range(HP):
                                do_scores((t - LAG1) * HP + u)
                        if 0 <= t - LAG2 < H // HP:
                            for u in range(HP):
                                do_pv((t - LAG2) * HP + u)
                    while len(res1) < NB:
                        res1.append(wo_part(len(res1), 0, KS_H, None))
                    res = jnp.concatenate([wo_part(j, KS_H, H, res1[j]) for j in range(NB)], axis=1)
                    mem = res[0:M].astype(BF16).astype(F32)
                    g1 = jnp.concatenate([1.0 - g] * NB, axis=1)
                    outb[pl.ds(r0 + M, SEG - M), :] = (g1 * res)[M:].astype(BF16)
                return mem

            lax.fori_loop(0, NPAIR, pair_body, mem0_ref[...].astype(F32), unroll=2)

            ER = EPI_SEGS * M
            ROWS = EPI_SEGS * SEG

            def epi_body(q, c):
                r0 = pl.multiple_of(q * ROWS, ROWS)
                od = [ld_bf(h * (R // 2) + q * (ER // 2), ER // 2, ER // 2) for h in range(H)]
                g = gm[pl.ds(r0, ROWS), :]
                for j in range(NB):
                    lo, hi = j * LANES, (j + 1) * LANES
                    res = None
                    for h in range(H):
                        t = _dot(od[h], wo_load(j, h * E, (h + 1) * E))
                        res = t if res is None else t + res
                    i0 = q * (ROWS // CH)
                    prev = ld_f32(UOFF + (j * NC + jnp.maximum(i0 - 1, 0)) * 2 * CH, 2 * CH, CH)
                    prev = jnp.where(i0 > 0, prev, 0.0)
                    ys = []
                    for i in range(ROWS // CH):
                        cur = ld_f32(UOFF + (j * NC + i0 + i) * 2 * CH, 2 * CH, CH)
                        zre = cur[0:HALF] - prev[CH:CH + HALF]
                        zro = cur[HALF:CH] + prev[CH + HALF:]
                        zie = cur[CH:CH + HALF] + prev[0:HALF]
                        zio = cur[CH + HALF:] - prev[HALF:CH]
                        ysum = _dot(inv_ref[0], jnp.concatenate([zre - zie, zro + zio], axis=0).astype(BF16))
                        ydif = _dot(inv_ref[1], jnp.concatenate([zre + zie, zro - zio], axis=0).astype(BF16))
                        ys += [ysum + ydif, _flip_rows(ysum - ydif)]
                        prev = cur
                    y = jnp.concatenate(ys, axis=0)
                    a = g * (x_v[pl.ds(r0, ROWS), lo:hi].astype(F32) * y)
                    parts = []
                    for sgm in range(EPI_SEGS):
                        s0 = sgm * SEG
                        parts.append((1.0 - g[s0:s0 + M]) * res[sgm * M:(sgm + 1) * M])
                        parts.append(outb[pl.ds(r0 + s0 + M, SEG - M), lo:hi].astype(F32))
                    outb[pl.ds(r0, ROWS), lo:hi] = (a + jnp.concatenate(parts, axis=0)).astype(BF16)
                    if (j + 1) % OUTJ == 0:
                        cp_out(q, hi - OUTJ * LANES, hi).start()
                return c
            lax.fori_loop(0, N_EPI, epi_body, 0, unroll=2)
            pltpu.make_async_copy(outb, out_hbm, sems.at[SOUT]).wait()

        pl.run_scoped(main, pltpu.VMEM((S, D), BF16))

    scratch = [
        pltpu.VMEM((S, D), BF16),
        pltpu.VMEM((3 * H + NB * WPJ, WROWS, LANES), U32),
        pltpu.VMEM((AROWS, LANES), U32),
        pltpu.VMEM((S, LANES), F32),
        pltpu.VMEM((NB, KS, LANES), BF16),
        pltpu.VMEM((NB, LANES), BF16),
        pltpu.VMEM((NB, LANES), BF16),
        pltpu.VMEM((M, D), BF16),
        pltpu.VMEM((2, 2 * CH, CH), BF16),
        pltpu.VMEM((2, CH // 2, CH), BF16),
        pltpu.SemaphoreType.DMA((n_sems,)),
    ]
    return kernel, scratch


@functools.partial(jax.jit, static_argnames=("B_seg_len",))
def pallas_gated_mix__ssm_conv_h3__memory_aug_recurrent_mem_tr__prompt_kernel(
    A_q: jax.Array,
    A_k: jax.Array,
    A_v: jax.Array,
    A_shift_k: jax.Array,
    A_ssm_k: jax.Array,
    A_ssm_D: jax.Array,
    B_x: jax.Array,
    B_mem0: jax.Array,
    B_Wq: jax.Array,
    B_Wk: jax.Array,
    B_Wv: jax.Array,
    B_Wo: jax.Array,
    B_seg_len: int,
    gate_w: jax.Array,
):
    B, S, D = A_q.shape
    assert B == 1
    H, E = B_Wq.shape[1], B_Wq.shape[2]
    M = B_mem0.shape[1]
    KS = A_shift_k.shape[1]
    NB = D // LANES
    kernel, scratch = _make_kernel(S, D, H, E, M, int(B_seg_len), KS)
    fwd, inv = _dft_mats()

    any_spec = pl.BlockSpec(memory_space=pl.ANY)
    out = pl.pallas_call(
        kernel,
        out_shape=jax.ShapeDtypeStruct((S, D), A_q.dtype),
        in_specs=[any_spec] * 15,
        out_specs=any_spec,
        scratch_shapes=scratch,
        compiler_params=pltpu.CompilerParams(vmem_limit_bytes=126 * 1024 * 1024,
                                             disable_bounds_checks=True,
                                             disable_semaphore_checks=True),
    )(
        A_q.reshape(S, D), A_q.reshape(S // int(B_seg_len), int(B_seg_len), D), A_k.reshape(S, D), A_v.reshape(S, D), A_ssm_k,
        B_Wq, B_Wk, B_Wv, B_Wo.reshape(H * E, D),
        A_shift_k.reshape(NB, LANES, KS).transpose(0, 2, 1), A_ssm_D.reshape(NB, LANES),
        gate_w.reshape(NB, LANES), B_mem0.reshape(M, D),
        jnp.asarray(fwd, dtype=BF16), jnp.asarray(inv, dtype=BF16),
    )
    return out.reshape(1, S, D)
```
